```python
import jax
import jax.numpy as jnp

def _softmax(x, axis=-1):
    return jax.nn.softmax(x, axis=axis)

def _gelu(x):
    return jax.nn.gelu(x, approximate=True)

def _silu(x):
    return jax.nn.silu(x)

def _sigmoid(x):
    return jax.nn.sigmoid(x)

def _layernorm(x, axis=-1, eps=1e-05):
    m = jnp.mean(x, axis=axis, keepdims=True)
    v = jnp.var(x, axis=axis, keepdims=True)
    return (x - m) / jnp.sqrt(v + eps)

def _scatter_add(tgt, idx, src, axis=0):
    return tgt.at[idx].add(src)

def _segment_sum(src, seg, n):
    return jax.ops.segment_sum(src, seg, n)

class _Rng:

    def __init__(self, key):
        self._k = key

    def _next(self):
        self._k, sub = jax.random.split(self._k)
        return sub

    def normal(self, shape):
        return jax.random.normal(self._next(), shape, dtype=jnp.bfloat16)

    def randint(self, lo, hi, shape):
        return jax.random.randint(self._next(), shape, lo, hi, dtype=jnp.int32)

    def uniform(self, shape, lo=0.0, hi=1.0):
        return jax.random.uniform(self._next(), shape, jnp.bfloat16, lo, hi)

    def permutation(self, n):
        return jax.random.permutation(self._next(), n)
kernel_name = 'adaLN_cond__sliding_block_cached__dense_activation_gelu__decode'

def setup_inputs():
    _rng = _Rng(jax.random.key(int.from_bytes(__import__("os").urandom(4), "little")))
    _w = lambda a: (lambda t: t.astype(jnp.bfloat16) if jnp.issubdtype(t.dtype, jnp.floating) else t)(jnp.asarray(a))

    def _A_setup():
        B, Sq, D = (4, 1, 640)
        Hq, Hkv, Sk, Dh = (32, 32, 8192, 128)
        assert Hq % Hkv == 0, (Hq, Hkv)
        return {'x': _w((lambda *s: _rng.normal(s) * 0.05)(B, Sq, D)), 'k_cache': _w((lambda *s: _rng.normal(s) * 0.05)(B, Hkv, Sk, Dh)), 'v_cache': _w((lambda *s: _rng.normal(s) * 0.05)(B, Hkv, Sk, Dh)), 'wq': _w((lambda *s: _rng.normal(s) * 0.05)(D, Hq * Dh) * D ** (-0.5)), 'wo': _w((lambda *s: _rng.normal(s) * 0.05)(Hq * Dh, D) * (Hq * Dh) ** (-0.5))}
    _A_in = _A_setup()

    def _B_setup():
        B, S, D, F = (4, 1, 640, 1728)
        return {'x': _w((lambda *s: _rng.normal(s) * 0.05)(B, S, D)), 'w1': _w((lambda *s: _rng.normal(s) * 0.05)(D, F) * D ** (-0.5)), 'b1': _w((lambda *s: _rng.normal(s) * 0.05)(F) * 0.01), 'w2': _w((lambda *s: _rng.normal(s) * 0.05)(F, D) * F ** (-0.5)), 'b2': _w((lambda *s: _rng.normal(s) * 0.05)(D) * 0.01)}
    _B_in = _B_setup()
    return {'A_x': _A_in['x'], 'A_k_cache': _A_in['k_cache'], 'A_v_cache': _A_in['v_cache'], 'A_wq': _A_in['wq'], 'A_wo': _A_in['wo'], 'B_x': _B_in['x'], 'B_w1': _B_in['w1'], 'B_b1': _B_in['b1'], 'B_w2': _B_in['w2'], 'B_b2': _B_in['b2'], 'c': _w((lambda *s: _rng.normal(s) * 0.05)(4, 640)), 'w_mod': _w((lambda *s: _rng.normal(s) * 0.05)(640, 6 * 640) * 640 ** (-0.5))}

def reference(A_x, A_k_cache, A_v_cache, A_wq, A_wo, B_x, B_w1, B_b1, B_w2, B_b2, c, w_mod):

    def _A_ref(x, k_cache, v_cache, wq, wo):
        B, Sq, D = x.shape
        Hq, Dh = (32, 128)
        Hkv, Sk = (k_cache.shape[1], k_cache.shape[2])
        W = min(4096, max(256, Sk // 4))
        rep = Hq // Hkv
        q = (lambda x, *d: x.transpose(*d))((x @ wq).reshape(B, Sq, Hq, Dh), 0, 2, 1, 3)
        k = jnp.repeat(k_cache[:, :, Sk - W:, :], rep, axis=1)
        v = jnp.repeat(v_cache[:, :, Sk - W:, :], rep, axis=1)
        scores = jnp.einsum('bhqd,bhkd->bhqk', q, k) * Dh ** (-0.5)
        p = _softmax(scores, axis=-1)
        o = jnp.einsum('bhqk,bhkd->bhqd', p, v)
        return (lambda x, *d: x.transpose(*d))(o, 0, 2, 1, 3).reshape(B, Sq, Hq * Dh) @ wo

    def _B_ref(x, w1, b1, w2, b2):
        h = jnp.einsum('bsd,df->bsf', x, w1) + b1
        h = _gelu(h)
        return jnp.einsum('bsf,fd->bsd', h, w2) + b2
    x = A_x
    mod = (_silu(c) @ w_mod).reshape(c.shape[0], 6, 1, -1)
    sa, ca, ga, sb, cb, gb = (mod[:, 0].copy(), mod[:, 1].copy(), mod[:, 2].copy(), mod[:, 3].copy(), mod[:, 4].copy(), mod[:, 5].copy())
    h = _layernorm(x, axis=-1) * (1 + ca) + sa
    x = x + ga * _A_ref(h, A_k_cache, A_v_cache, A_wq, A_wo)
    h = _layernorm(x, axis=-1) * (1 + cb) + sb
    x = x + gb * _B_ref(h, B_w1, B_b1, B_w2, B_b2)
    return x
```

```python
import functools
import jax
import jax.numpy as jnp
from jax import lax
import jax.experimental.pallas as pl
import jax.experimental.pallas.tpu as pltpu

B, D, H, SK, DH, F = 4, 640, 32, 8192, 128, 1728
W = 2048
NBUF = 3
EPS = 1e-5
SCALE = DH ** -0.5
f32 = jnp.float32
bf16 = jnp.bfloat16


def _ln(x):
    m = jnp.mean(x, axis=-1, keepdims=True)
    xc = x - m
    v = jnp.mean(xc * xc, axis=-1, keepdims=True)
    return xc * lax.rsqrt(v + EPS)


def _kernel(x_hbm, k_hbm, v_hbm, wq_hbm, wo_hbm, w1t_hbm, b1_hbm, w2_hbm, b2_hbm, c_hbm, wmod_hbm,
            o_ref,
            kbuf, vbuf, wq_v, wo_v, w1t_v, w2_v, wmod_v, x_v, c_v, b1_v, b2_v, q_scr, o_scr,
            ksem, vsem, wsem):
    def kv_copies(h, slot):
        return (pltpu.make_async_copy(k_hbm.at[:, h, pl.ds(SK - W, W), :], kbuf.at[slot], ksem.at[slot]),
                pltpu.make_async_copy(v_hbm.at[:, h, pl.ds(SK - W, W), :], vbuf.at[slot], vsem.at[slot]))

    c_cp = pltpu.make_async_copy(c_hbm, c_v, wsem.at[0])
    x_cp = pltpu.make_async_copy(x_hbm, x_v, wsem.at[1])
    wmod_cp = pltpu.make_async_copy(wmod_hbm, wmod_v, wsem.at[2])
    wq_cp = pltpu.make_async_copy(wq_hbm, wq_v, wsem.at[3])
    wo_cp = pltpu.make_async_copy(wo_hbm, wo_v, wsem.at[4])
    w1_cp = pltpu.make_async_copy(w1t_hbm, w1t_v, wsem.at[5])
    w2_cp = pltpu.make_async_copy(w2_hbm, w2_v, wsem.at[6])
    b1_cp = pltpu.make_async_copy(b1_hbm, b1_v, wsem.at[7])
    b2_cp = pltpu.make_async_copy(b2_hbm, b2_v, wsem.at[8])
    for cp in (c_cp, x_cp, b1_cp, b2_cp, wmod_cp, wq_cp):
        cp.start()
    for s in range(NBUF):
        for cp in kv_copies(s, s):
            cp.start()

    c_cp.wait(); x_cp.wait(); wmod_cp.wait()
    c = c_v[...].astype(f32)
    sc = (c * jax.nn.sigmoid(c)).astype(bf16)
    mod = jnp.dot(sc, wmod_v[...], preferred_element_type=f32)
    x = x_v[...].astype(f32)
    h = _ln(x) * (1.0 + mod[:, D:2 * D]) + mod[:, 0:D]
    wq_cp.wait()
    q = jnp.dot(h.astype(bf16), wq_v[...], preferred_element_type=f32)
    for hh in range(H):
        q_scr[hh] = q[:, hh * DH:(hh + 1) * DH].astype(bf16)

    row = lax.broadcasted_iota(jnp.int32, (B, DH), 0)

    def step(hh, carry):
        slot = hh % NBUF
        kc, vc = kv_copies(hh, slot)
        kc.wait()
        vc.wait()
        qh = q_scr[hh]
        o = jnp.zeros((B, DH), f32)
        for b in range(B):
            s = lax.dot_general(qh, kbuf[slot, b], (((1,), (1,)), ((), ())), preferred_element_type=f32)
            m = jnp.max(s, axis=-1, keepdims=True)
            p = jnp.exp((s - m) * SCALE)
            l = jnp.sum(p, axis=-1, keepdims=True)
            ob = jnp.dot(p.astype(bf16), vbuf[slot, b], preferred_element_type=f32)
            o = jnp.where(row == b, ob / l, o)
        o_scr[hh] = o

        @pl.when(hh + NBUF < H)
        def _():
            for cp in kv_copies(hh + NBUF, slot):
                cp.start()

        @pl.when(hh == H - NBUF)
        def _():
            for cp in (wo_cp, w1_cp, w2_cp):
                cp.start()
        return carry

    lax.fori_loop(0, H, step, 0)

    o_all = jnp.concatenate([o_scr[hh] for hh in range(H)], axis=-1).astype(bf16)
    wo_cp.wait()
    attn = jnp.dot(o_all, wo_v[...], preferred_element_type=f32)
    x1 = x + mod[:, 2 * D:3 * D] * attn
    h2 = _ln(x1) * (1.0 + mod[:, 4 * D:5 * D]) + mod[:, 3 * D:4 * D]
    w1_cp.wait(); b1_cp.wait()
    u = lax.dot_general(h2.astype(bf16), w1t_v[...], (((1,), (1,)), ((), ())), preferred_element_type=f32)
    u = u + b1_v[...].astype(f32).reshape(1, F)
    g = jax.nn.gelu(u, approximate=True)
    w2_cp.wait(); b2_cp.wait()
    y = jnp.dot(g.astype(bf16), w2_v[...], preferred_element_type=f32) + b2_v[...].astype(f32).reshape(1, D)
    o_ref[...] = (x1 + mod[:, 5 * D:6 * D] * y).astype(o_ref.dtype)


@jax.jit
def pallas_adaLN_cond__sliding_block_cached__dense_activation_gelu__decode_kernel(A_x, A_k_cache, A_v_cache, A_wq, A_wo, B_x, B_w1, B_b1, B_w2, B_b2, c, w_mod):
    out = pl.pallas_call(
        _kernel,
        in_specs=[pl.BlockSpec(memory_space=pl.ANY)] * 11,
        out_specs=pl.BlockSpec(memory_space=pltpu.VMEM),
        out_shape=jax.ShapeDtypeStruct((B, D), bf16),
        scratch_shapes=[
            pltpu.VMEM((NBUF, B, W, DH), bf16), pltpu.VMEM((NBUF, B, W, DH), bf16),
            pltpu.VMEM((D, H * DH), bf16), pltpu.VMEM((H * DH, D), bf16),
            pltpu.VMEM((F, D), bf16), pltpu.VMEM((F, D), bf16), pltpu.VMEM((D, 6 * D), bf16),
            pltpu.VMEM((B, D), bf16), pltpu.VMEM((B, D), bf16),
            pltpu.VMEM((F,), bf16), pltpu.VMEM((D,), bf16),
            pltpu.VMEM((H, B, DH), bf16), pltpu.VMEM((H, B, DH), f32),
            pltpu.SemaphoreType.DMA((NBUF,)), pltpu.SemaphoreType.DMA((NBUF,)), pltpu.SemaphoreType.DMA((9,)),
        ],
        compiler_params=pltpu.CompilerParams(vmem_limit_bytes=100 * 1024 * 1024, disable_bounds_checks=True),
    )(A_x.reshape(B, D), A_k_cache, A_v_cache, A_wq, A_wo, B_w1.T, B_b1, B_w2, B_b2, c, w_mod)
    return out.reshape(B, 1, D)
```

```python
import functools
import jax
import jax.numpy as jnp
from jax import lax
import jax.experimental.pallas as pl
import jax.experimental.pallas.tpu as pltpu

B, D, H, SK, DH, F = 4, 640, 32, 8192, 128, 1728
W = 2048
EPS = 1e-5
SCALE = DH ** -0.5
f32 = jnp.float32
bf16 = jnp.bfloat16


def _ln(x):
    m = jnp.mean(x, axis=-1, keepdims=True)
    xc = x - m
    v = jnp.mean(xc * xc, axis=-1, keepdims=True)
    return xc * lax.rsqrt(v + EPS)


def make(G=8, R=16, NBUF=3, LOOK=2, WROWS=24, WOR=16, W2SPLIT=(896, 1536), NOATT=False, NOTAIL=False, UNROLL=1):
    NJ = W // R
    PER = NJ // G
    NSTEP = B * H // G
    NIT = B * H
    NT = LOOK * G
    WO_PER = (H * DH // 2) // NT

    def chunks(src, dst, sem, r0, r1, rstep, c0, c1, cstep):
        out = []
        for r in range(r0, r1, rstep):
            rs = min(rstep, r1 - r)
            for c in range(c0, c1, cstep):
                cs = min(cstep, c1 - c)
                out.append((src.at[pl.ds(r, rs), pl.ds(c, cs)], dst.at[pl.ds(r, rs), pl.ds(c, cs)], sem))
        return out

    def inter(a, b):
        out = []; i = j = 0
        while i < len(a) or j < len(b):
            if j >= len(b) or (i < len(a) and i * len(b) <= j * len(a)):
                out.append(a[i] + (0,)); i += 1
            else:
                out.append(b[j] + (1,)); j += 1
        return out

    def order2(lst):
        h = (len(lst) + 1) // 2
        return inter(lst[:h], lst[h:])

    def issue(lst):
        for s, d, sem, p in lst:
            pltpu.make_async_copy(s, d, sem).start(priority=p)

    def waitbuf(view, sem):
        pltpu.make_async_copy(view, view, sem).wait()

    def _kernel(x_hbm, k_hbm, v_hbm, wq_hbm, wo_hbm, w1t_hbm, b1_hbm, w2_hbm, b2_hbm, c_hbm, wmod_hbm,
                o_ref,
                kbuf, vbuf, wq_v, wo_v, w1t_v, w2_v, wmod_v, x_v, c_v, b1_v, b2_v, q_scr, o_scr,
                ksem, vsem, wsem):
        def kv_issue(step, slot, row0, n):
            for j in range(n):
                r = row0 + j * R
                if not isinstance(r, int):
                    r = pl.multiple_of(r, R)
                pltpu.make_async_copy(k_hbm.at[step, :, pl.ds(SK - W + r, R), :],
                                      kbuf.at[slot, :, pl.ds(r, R), :], ksem.at[slot]).start(priority=0)
                pltpu.make_async_copy(v_hbm.at[step, :, pl.ds(SK - W + r, R), :],
                                      vbuf.at[slot, :, pl.ds(r, R), :], vsem.at[slot]).start(priority=1)

        c_cp = pltpu.make_async_copy(c_hbm, c_v, wsem.at[0])
        x_cp = pltpu.make_async_copy(x_hbm, x_v, wsem.at[1])
        b1_cp = pltpu.make_async_copy(b1_hbm, b1_v, wsem.at[2])
        b2_cp = pltpu.make_async_copy(b2_hbm, b2_v, wsem.at[3])
        wmod_l = order2(chunks(wmod_hbm, wmod_v, wsem.at[4], 0, D, 8, 0, 6 * D, 3 * D))
        wq_l = order2(chunks(wq_hbm, wq_v, wsem.at[5], 0, D, 8, 0, H * DH, 2048))
        w1_l = order2(chunks(w1t_hbm, w1t_v, wsem.at[7], 0, F, WROWS, 0, D, D))
        s0, s1 = W2SPLIT
        w2_l = inter(chunks(w2_hbm, w2_v, wsem.at[8], 0, s0, WROWS, 0, D, D),
                     chunks(w2_hbm, w2_v, wsem.at[9], s0, s1, WROWS, 0, D, D)
                     + chunks(w2_hbm, w2_v, wsem.at[10], s1, F, WROWS, 0, D, D))

        issue(wmod_l)
        for cp in (c_cp, x_cp, b1_cp, b2_cp):
            cp.start()
        issue(wq_l)
        c_cp.wait(); x_cp.wait()
        waitbuf(wmod_v, wsem.at[4])
        c = c_v[...].astype(f32)
        sc = (c * jax.nn.sigmoid(c)).astype(bf16)
        mod = jnp.dot(sc, wmod_v[...], preferred_element_type=f32)
        x = x_v[...].astype(f32)
        h = (_ln(x) * (1.0 + mod[:, D:2 * D]) + mod[:, 0:D]).astype(bf16)
        kv_issue(0, 0, 0, NJ // 2)
        waitbuf(wq_v, wsem.at[5])
        q = jnp.dot(h, wq_v[...], preferred_element_type=f32)
        for hh in range(H):
            q_scr[hh] = q[:, hh * DH:(hh + 1) * DH].astype(bf16)
        o_scr[...] = jnp.zeros_like(o_scr)
        kv_issue(0, 0, (NJ // 2) * R, NJ // 2)
        for s in range(1, LOOK):
            kv_issue(s, s, 0, NJ)

        row = lax.broadcasted_iota(jnp.int32, (B, DH), 0)

        def body(i, carry):
            step = i // G
            g = i % G
            slot = step % NBUF
            b = i // H
            hh = i % H

            @pl.when(i < NIT - NT)
            def _():
                kv_issue(step + LOOK, (step + LOOK) % NBUF, g * (PER * R), PER)

            @pl.when(i >= NIT - NT)
            def _():
                t = i - (NIT - NT)
                for j in range(0, WO_PER, WOR):
                    for p in range(2):
                        r = pl.multiple_of(p * (H * DH // 2) + t * WO_PER + j, WOR)
                        pltpu.make_async_copy(wo_hbm.at[pl.ds(r, WOR), :], wo_v.at[pl.ds(r, WOR), :],
                                              wsem.at[6]).start(priority=p)

            @pl.when(g == 0)
            def _():
                waitbuf(kbuf.at[slot], ksem.at[slot])
                waitbuf(vbuf.at[slot], vsem.at[slot])

            if NOATT:
                return carry
            qh = q_scr[hh]
            s = lax.dot_general(qh, kbuf[slot, g], (((1,), (1,)), ((), ())), preferred_element_type=f32)
            m = jnp.max(s, axis=-1, keepdims=True)
            p = jnp.exp((s - m) * SCALE)
            l = jnp.sum(p, axis=-1, keepdims=True)
            ob = jnp.dot(p.astype(bf16), vbuf[slot, g], preferred_element_type=f32)
            o_scr[hh] = jnp.where(row == b, ob / l, o_scr[hh])
            return carry

        lax.fori_loop(0, NIT, body, 0, unroll=UNROLL)

        issue(w1_l)
        if NOTAIL:
            issue(w2_l)
            waitbuf(wo_v, wsem.at[6]); waitbuf(w1t_v, wsem.at[7]); b1_cp.wait(); b2_cp.wait()
            waitbuf(w2_v.at[pl.ds(0, s0)], wsem.at[8]); waitbuf(w2_v.at[pl.ds(s0, s1 - s0)], wsem.at[9])
            waitbuf(w2_v.at[pl.ds(s1, F - s1)], wsem.at[10])
            o_ref[...] = x.astype(o_ref.dtype)
            return
        o_all = jnp.concatenate([o_scr[hh] for hh in range(H)], axis=-1).astype(bf16)
        waitbuf(wo_v, wsem.at[6])
        attn = jnp.dot(o_all, wo_v[...], preferred_element_type=f32)
        x1 = x + mod[:, 2 * D:3 * D] * attn
        h2 = (_ln(x1) * (1.0 + mod[:, 4 * D:5 * D]) + mod[:, 3 * D:4 * D]).astype(bf16)
        issue(w2_l)
        b1_cp.wait(); b2_cp.wait()
        waitbuf(w1t_v, wsem.at[7])
        u = lax.dot_general(h2, w1t_v[...], (((1,), (1,)), ((), ())), preferred_element_type=f32)
        u = u + b1_v[...].astype(f32).reshape(1, F)
        g = jax.nn.gelu(u, approximate=True).astype(bf16)
        y = b2_v[...].astype(f32).reshape(1, D)
        for (r0, r1, k) in ((0, s0, 8), (s0, s1, 9), (s1, F, 10)):
            waitbuf(w2_v.at[pl.ds(r0, r1 - r0)], wsem.at[k])
            y = y + jnp.dot(g[:, r0:r1], w2_v[r0:r1, :], preferred_element_type=f32)
        o_ref[...] = (x1 + mod[:, 5 * D:6 * D] * y).astype(o_ref.dtype)

    @jax.jit
    def kernel(A_x, A_k_cache, A_v_cache, A_wq, A_wo, B_x, B_w1, B_b1, B_w2, B_b2, c, w_mod):
        out = pl.pallas_call(
            _kernel,
            in_specs=[pl.BlockSpec(memory_space=pl.ANY)] * 11,
            out_specs=pl.BlockSpec(memory_space=pltpu.VMEM),
            out_shape=jax.ShapeDtypeStruct((B, D), bf16),
            scratch_shapes=[
                pltpu.VMEM((NBUF, G, W, DH), bf16), pltpu.VMEM((NBUF, G, W, DH), bf16),
                pltpu.VMEM((D, H * DH), bf16), pltpu.VMEM((H * DH, D), bf16),
                pltpu.VMEM((F, D), bf16), pltpu.VMEM((F, D), bf16), pltpu.VMEM((D, 6 * D), bf16),
                pltpu.VMEM((B, D), bf16), pltpu.VMEM((B, D), bf16),
                pltpu.VMEM((F,), bf16), pltpu.VMEM((D,), bf16),
                pltpu.VMEM((H, B, DH), bf16), pltpu.VMEM((H, B, DH), f32),
                pltpu.SemaphoreType.DMA((NBUF,)), pltpu.SemaphoreType.DMA((NBUF,)), pltpu.SemaphoreType.DMA((11,)),
            ],
            compiler_params=pltpu.CompilerParams(vmem_limit_bytes=100 * 1024 * 1024, disable_bounds_checks=True),
        )(A_x.reshape(B, D), A_k_cache.reshape(NSTEP, G, SK, DH), A_v_cache.reshape(NSTEP, G, SK, DH),
          A_wq, A_wo, B_w1.T, B_b1, B_w2, B_b2, c, w_mod)
        return out.reshape(B, 1, D)
    return kernel

pallas_adaLN_cond__sliding_block_cached__dense_activation_gelu__decode_kernel = make()
```

```python
import jax
import jax.numpy as jnp
from jax import lax
import jax.experimental.pallas as pl
import jax.experimental.pallas.tpu as pltpu

_F32 = jnp.float32
_BF16 = jnp.bfloat16
_EPS = 1e-5

_HEADS = 32
_DH = 128
_G = 8
_R = 16
_NBUF = 3
_LOOK = 2
_NSTREAM = 4
_WO_ROWS = 16
_FF_ROWS = 24
_W2_SPLIT = (896, 1536)

_S_KV = 0
_S_C, _S_X, _S_B1, _S_B2, _S_MOD, _S_Q, _S_O, _S_W1, _S_W2 = range(_NBUF, _NBUF + 9)
_NSEM = _S_W2 + len(_W2_SPLIT) + 1


def _layernorm(x):
    m = jnp.mean(x, axis=-1, keepdims=True)
    xc = x - m
    v = jnp.mean(xc * xc, axis=-1, keepdims=True)
    return xc * lax.rsqrt(v + _EPS)


def _chunks(src, dst, sem, r0, r1, rstep, cstep):
    ncols = src.shape[1]
    out = []
    for r in range(r0, r1, rstep):
        for c in range(0, ncols, cstep):
            idx = (pl.ds(r, min(rstep, r1 - r)), pl.ds(c, min(cstep, ncols - c)))
            out.append((src.at[idx], dst.at[idx], sem))
    return out


def _round_robin(lst, n):
    parts = [lst[(len(lst) * s) // n:(len(lst) * (s + 1)) // n] for s in range(n)]
    return [p[i] for i in range(max(map(len, parts))) for p in parts if i < len(p)]


def _alternate(a, b):
    out, i, j = [], 0, 0
    while i < len(a) or j < len(b):
        if j >= len(b) or (i < len(a) and i * len(b) <= j * len(a)):
            out.append(a[i] + (0,))
            i += 1
        else:
            out.append(b[j] + (1,))
            j += 1
    return out


def _two_queues(lst, nstream):
    h = (len(lst) + 1) // 2
    return _alternate(_round_robin(lst[:h], nstream), _round_robin(lst[h:], nstream))


def _start(copies):
    for src, dst, sem, queue in copies:
        pltpu.make_async_copy(src, dst, sem).start(priority=queue)


def _wait_filled(view, sem):
    pltpu.make_async_copy(view, view, sem).wait()


def _kernel(x_hbm, k_hbm, v_hbm, wq_hbm, wo_hbm, w1t_hbm, b1_hbm, w2_hbm, b2_hbm, c_hbm, wmod_hbm,
            o_ref,
            kv_buf, wq_v, wo_v, w1t_v, w2_v, wmod_v, x_v, c_v, b1_v, b2_v, q_scr, o_scr, sem):
    nb, d = x_v.shape
    ff = w2_v.shape[0]
    win = kv_buf.shape[3]
    row0 = k_hbm.shape[2] - win
    n_desc = win // _R
    per_it = n_desc // _G
    n_it = nb * _HEADS
    n_tail = _LOOK * _G
    scale = _DH ** -0.5

    def start_kv(step, slot, r_first, n):
        for j in range(n):
            r = r_first + j * _R
            if not isinstance(r, int):
                r = pl.multiple_of(r, _R)
            for queue, src in enumerate((k_hbm, v_hbm)):
                pltpu.make_async_copy(src.at[step, :, pl.ds(row0 + r, _R), :],
                                      kv_buf.at[slot, queue, :, pl.ds(r, _R), :],
                                      sem.at[_S_KV + slot]).start(priority=queue)

    c_cp = pltpu.make_async_copy(c_hbm, c_v, sem.at[_S_C])
    x_cp = pltpu.make_async_copy(x_hbm, x_v, sem.at[_S_X])
    b1_cp = pltpu.make_async_copy(b1_hbm, b1_v, sem.at[_S_B1])
    b2_cp = pltpu.make_async_copy(b2_hbm, b2_v, sem.at[_S_B2])

    _start(_two_queues(_chunks(wmod_hbm, wmod_v, sem.at[_S_MOD], 0, d, 8, 3 * d), _NSTREAM))
    for cp in (c_cp, x_cp, b1_cp, b2_cp):
        cp.start()
    _start(_two_queues(_chunks(wq_hbm, wq_v, sem.at[_S_Q], 0, d, 8, _HEADS * _DH // 2), _NSTREAM))

    c_cp.wait()
    x_cp.wait()
    _wait_filled(wmod_v, sem.at[_S_MOD])
    c = c_v[...].astype(_F32)
    mod = jnp.dot((c * jax.nn.sigmoid(c)).astype(_BF16), wmod_v[...], preferred_element_type=_F32)
    sa, ca, ga, sb, cb, gb = (mod[:, k * d:(k + 1) * d] for k in range(6))
    x = x_v[...].astype(_F32)
    h = (_layernorm(x) * (1.0 + ca) + sa).astype(_BF16)

    start_kv(0, 0, 0, n_desc // 2)
    _wait_filled(wq_v, sem.at[_S_Q])
    q = jnp.dot(h, wq_v[...], preferred_element_type=_F32)
    for hh in range(_HEADS):
        q_scr[hh] = q[:, hh * _DH:(hh + 1) * _DH].astype(_BF16)
    o_scr[...] = jnp.zeros_like(o_scr)
    start_kv(0, 0, (n_desc // 2) * _R, n_desc // 2)
    for s in range(1, _LOOK):
        start_kv(s, s, 0, n_desc)

    batch_row = lax.broadcasted_iota(jnp.int32, (nb, _DH), 0)
    wo_half = _HEADS * _DH // 2
    wo_stream = wo_half // _NSTREAM
    wo_per_it = wo_stream // n_tail

    def attend(i, carry):
        step = i // _G
        g = i % _G
        slot = step % _NBUF

        @pl.when(i < n_it - n_tail)
        def _():
            start_kv(step + _LOOK, (step + _LOOK) % _NBUF, g * (per_it * _R), per_it)

        @pl.when(i >= n_it - n_tail)
        def _():
            t = i - (n_it - n_tail)
            for j in range(0, wo_per_it, _WO_ROWS):
                for s in range(_NSTREAM):
                    for queue in range(2):
                        r = queue * wo_half + s * wo_stream + t * wo_per_it + j
                        rows = pl.ds(pl.multiple_of(r, _WO_ROWS), _WO_ROWS)
                        pltpu.make_async_copy(wo_hbm.at[rows, :], wo_v.at[rows, :],
                                              sem.at[_S_O]).start(priority=queue)

        @pl.when(g == 0)
        def _():
            _wait_filled(kv_buf.at[slot], sem.at[_S_KV + slot])

        hh = i % _HEADS
        s = lax.dot_general(q_scr[hh], kv_buf[slot, 0, g], (((1,), (1,)), ((), ())),
                            preferred_element_type=_F32)
        p = jnp.exp((s - jnp.max(s, axis=-1, keepdims=True)) * scale)
        denom = jnp.sum(p, axis=-1, keepdims=True)
        o = jnp.dot(p.astype(_BF16), kv_buf[slot, 1, g], preferred_element_type=_F32)
        o_scr[hh] = jnp.where(batch_row == i // _HEADS, o / denom, o_scr[hh])
        return carry

    lax.fori_loop(0, n_it, attend, 0)

    _start(_two_queues(_chunks(w1t_hbm, w1t_v, sem.at[_S_W1], 0, ff, _FF_ROWS, d), 2))
    o_all = jnp.concatenate([o_scr[hh] for hh in range(_HEADS)], axis=-1).astype(_BF16)
    b1_cp.wait()
    b2_cp.wait()
    _wait_filled(wo_v, sem.at[_S_O])
    x1 = x + ga * jnp.dot(o_all, wo_v[...], preferred_element_type=_F32)
    h2 = (_layernorm(x1) * (1.0 + cb) + sb).astype(_BF16)

    bounds = (0,) + _W2_SPLIT + (ff,)
    w2_parts = [(bounds[k], bounds[k + 1], sem.at[_S_W2 + k]) for k in range(len(bounds) - 1)]
    w2_copies = [_chunks(w2_hbm, w2_v, sm, r0, r1, _FF_ROWS, d) for r0, r1, sm in w2_parts]
    _start(_alternate(w2_copies[0], sum(w2_copies[1:], [])))

    _wait_filled(w1t_v, sem.at[_S_W1])
    u = lax.dot_general(h2, w1t_v[...], (((1,), (1,)), ((), ())), preferred_element_type=_F32)
    u = u + b1_v[...].astype(_F32).reshape(1, ff)
    act = jax.nn.gelu(u, approximate=True).astype(_BF16)
    y = b2_v[...].astype(_F32).reshape(1, d)
    for r0, r1, sm in w2_parts:
        _wait_filled(w2_v.at[pl.ds(r0, r1 - r0)], sm)
        y = y + jnp.dot(act[:, r0:r1], w2_v[r0:r1, :], preferred_element_type=_F32)
    o_ref[...] = (x1 + gb * y).astype(o_ref.dtype)


@jax.jit
def pallas_adaLN_cond__sliding_block_cached__dense_activation_gelu__decode_kernel(
    A_x: jax.Array,
    A_k_cache: jax.Array,
    A_v_cache: jax.Array,
    A_wq: jax.Array,
    A_wo: jax.Array,
    B_x: jax.Array,
    B_w1: jax.Array,
    B_b1: jax.Array,
    B_w2: jax.Array,
    B_b2: jax.Array,
    c: jax.Array,
    w_mod: jax.Array,
):
    del B_x
    nb, sq, d = A_x.shape
    _, hkv, sk, dh = A_k_cache.shape
    ff = B_w2.shape[0]
    assert sq == 1 and hkv == _HEADS and dh == _DH
    win = min(4096, max(256, sk // 4))
    n_step = nb * hkv // _G

    out = pl.pallas_call(
        _kernel,
        in_specs=[pl.BlockSpec(memory_space=pl.ANY)] * 11,
        out_specs=pl.BlockSpec(memory_space=pltpu.VMEM),
        out_shape=jax.ShapeDtypeStruct((nb, d), A_x.dtype),
        scratch_shapes=[
            pltpu.VMEM((_NBUF, 2, _G, win, dh), _BF16),
            pltpu.VMEM((d, hkv * dh), _BF16),
            pltpu.VMEM((hkv * dh, d), _BF16),
            pltpu.VMEM((ff, d), _BF16),
            pltpu.VMEM((ff, d), _BF16),
            pltpu.VMEM((d, 6 * d), _BF16),
            pltpu.VMEM((nb, d), _BF16),
            pltpu.VMEM((nb, d), _BF16),
            pltpu.VMEM((ff,), _BF16),
            pltpu.VMEM((d,), _BF16),
            pltpu.VMEM((hkv, nb, dh), _BF16),
            pltpu.VMEM((hkv, nb, dh), _F32),
            pltpu.SemaphoreType.DMA((_NSEM,)),
        ],
        compiler_params=pltpu.CompilerParams(
            vmem_limit_bytes=64 * 1024 * 1024,
            disable_bounds_checks=True,
            disable_semaphore_checks=True,
        ),
    )(
        A_x.reshape(nb, d),
        A_k_cache.reshape(n_step, _G, sk, dh),
        A_v_cache.reshape(n_step, _G, sk, dh),
        A_wq, A_wo, B_w1.T, B_b1, B_w2, B_b2, c, w_mod,
    )
    return out.reshape(nb, 1, d)
```

```python
import jax
import jax.numpy as jnp
from jax import lax
import jax.experimental.pallas as pl
import jax.experimental.pallas.tpu as pltpu

_F32 = jnp.float32
_BF16 = jnp.bfloat16
_EPS = 1e-5

_HEADS = 32
_DH = 128
_G = 8
_R = 16
_NBUF = 3
_LOOK = 2
_NSTREAM = 4
_WO_ROWS = 16
_FF_ROWS = 16
_FF_CHUNKS = (288, 96, 48)

_S_KV = 0
_S_C, _S_X, _S_B1, _S_B2, _S_MOD, _S_Q, _S_O, _S_W1A, _S_W1B, _S_W2 = range(_NBUF, _NBUF + 10)
_NSEM = _S_W2 + len(_FF_CHUNKS)


def _layernorm(x):
    m = jnp.mean(x, axis=-1, keepdims=True)
    xc = x - m
    v = jnp.mean(xc * xc, axis=-1, keepdims=True)
    return xc * lax.rsqrt(v + _EPS)


def _chunks(src, dst, sem, rstep, cstep):
    nrows, ncols = src.shape
    out = []
    for r in range(0, nrows, rstep):
        for c in range(0, ncols, cstep):
            idx = (pl.ds(r, rstep), pl.ds(c, cstep))
            out.append((src.at[idx], dst.at[idx], sem))
    return out


def _round_robin(lst, n):
    parts = [lst[(len(lst) * s) // n:(len(lst) * (s + 1)) // n] for s in range(n)]
    return [p[i] for i in range(max(map(len, parts))) for p in parts if i < len(p)]


def _alternate(a, b):
    assert len(a) == len(b)
    return [t for x, y in zip(a, b) for t in (x + (0,), y + (1,))]


def _two_queues(lst):
    h = len(lst) // 2
    return _alternate(_round_robin(lst[:h], _NSTREAM), _round_robin(lst[h:], _NSTREAM))


def _start(copies):
    for src, dst, sem, queue in copies:
        pltpu.make_async_copy(src, dst, sem).start(priority=queue)


def _wait_filled(view, sem):
    pltpu.make_async_copy(view, view, sem).wait()


def _kernel(x_hbm, k_hbm, v_hbm, wq_hbm, wo_hbm, w1t_hbm, b1_hbm, w2_hbm, b2_hbm, c_hbm, wmod_hbm,
            o_ref,
            kv_buf, wq_v, wo_v, w1t_v, w2_v, wmod_v, x_v, c_v, b1_v, b2_v, b1_perm, q_scr, o_scr, sem):
    nb, d = x_v.shape
    ff = w2_v.shape[0]
    win = kv_buf.shape[3]
    row0 = k_hbm.shape[2] - win
    n_desc = win // _R
    per_it = n_desc // _G
    n_it = nb * _HEADS
    n_tail = _LOOK * _G
    scale = _DH ** -0.5

    def start_kv(step, slot, r_first, n):
        for j in range(n):
            r = r_first + j * _R
            if not isinstance(r, int):
                r = pl.multiple_of(r, _R)
            for which, src in enumerate((k_hbm, v_hbm)):
                pltpu.make_async_copy(src.at[step, :, pl.ds(row0 + r, _R), :],
                                      kv_buf.at[slot, which, :, pl.ds(r, _R), :],
                                      sem.at[_S_KV + slot]).start(priority=1 - which)

    ff_stream = ff // _NSTREAM
    assert sum(_FF_CHUNKS) == ff_stream
    ff_pos = [_NSTREAM * sum(_FF_CHUNKS[:k]) for k in range(len(_FF_CHUNKS) + 1)]

    def ff_rows(k, s):
        return s * ff_stream + sum(_FF_CHUNKS[:k]), ff_pos[k] + s * _FF_CHUNKS[k]

    def ff_copies(src, dst, sems):
        out = []
        for k, n in enumerate(_FF_CHUNKS):
            for j in range(0, n, _FF_ROWS):
                for s in range(_NSTREAM):
                    r_src, r_dst = ff_rows(k, s)
                    out.append((src.at[pl.ds(r_src + j, _FF_ROWS), :], dst.at[pl.ds(r_dst + j, _FF_ROWS), :],
                                sems[k]))
        return out

    c_cp = pltpu.make_async_copy(c_hbm, c_v, sem.at[_S_C])
    x_cp = pltpu.make_async_copy(x_hbm, x_v, sem.at[_S_X])
    b1_cp = pltpu.make_async_copy(b1_hbm, b1_v, sem.at[_S_B1])
    b2_cp = pltpu.make_async_copy(b2_hbm, b2_v, sem.at[_S_B2])

    _start(_two_queues(_chunks(wmod_hbm, wmod_v, sem.at[_S_MOD], 8, 3 * d)))
    for cp in (c_cp, x_cp, b1_cp, b2_cp):
        cp.start()
    _start(_two_queues(_chunks(wq_hbm, wq_v, sem.at[_S_Q], 8, _HEADS * _DH // 2)))

    c_cp.wait()
    x_cp.wait()
    b1_cp.wait()
    _wait_filled(wmod_v, sem.at[_S_MOD])
    b1 = b1_v[...].astype(_F32).reshape(1, ff)
    for k, n in enumerate(_FF_CHUNKS):
        for s in range(_NSTREAM):
            r_src, r_dst = ff_rows(k, s)
            b1_perm[:, r_dst:r_dst + n] = b1[:, r_src:r_src + n]
    c = c_v[...].astype(_F32)
    mod = jnp.dot((c * jax.nn.sigmoid(c)).astype(_BF16), wmod_v[...], preferred_element_type=_F32)
    sa, ca, ga, sb, cb, gb = (mod[:, k * d:(k + 1) * d] for k in range(6))
    x = x_v[...].astype(_F32)
    h = (_layernorm(x) * (1.0 + ca) + sa).astype(_BF16)

    start_kv(0, 0, 0, n_desc // 2)
    _wait_filled(wq_v, sem.at[_S_Q])
    q = jnp.dot(h, wq_v[...], preferred_element_type=_F32)
    for hh in range(_HEADS):
        q_scr[hh] = q[:, hh * _DH:(hh + 1) * _DH].astype(_BF16)
    o_scr[...] = jnp.zeros_like(o_scr)
    start_kv(0, 0, (n_desc // 2) * _R, n_desc // 2)
    for s in range(1, _LOOK):
        start_kv(s, s, 0, n_desc)

    batch_row = lax.broadcasted_iota(jnp.int32, (nb, _DH), 0)
    wo_half = _HEADS * _DH // 2
    wo_stream = wo_half // _NSTREAM
    wo_per_it = wo_stream // n_tail

    def attend(i, carry):
        step = i // _G
        g = i % _G
        slot = step % _NBUF

        @pl.when(i < n_it - n_tail)
        def _():
            start_kv(step + _LOOK, (step + _LOOK) % _NBUF, g * (per_it * _R), per_it)

        @pl.when(i >= n_it - n_tail)
        def _():
            t = i - (n_it - n_tail)
            for j in range(0, wo_per_it, _WO_ROWS):
                for s in range(_NSTREAM):
                    for queue in range(2):
                        r = queue * wo_half + s * wo_stream + t * wo_per_it + j
                        rows = pl.ds(pl.multiple_of(r, _WO_ROWS), _WO_ROWS)
                        pltpu.make_async_copy(wo_hbm.at[rows, :], wo_v.at[rows, :],
                                              sem.at[_S_O]).start(priority=queue)

        @pl.when(g == 0)
        def _():
            _wait_filled(kv_buf.at[slot], sem.at[_S_KV + slot])

        hh = i % _HEADS
        s = lax.dot_general(q_scr[hh], kv_buf[slot, 0, g], (((1,), (1,)), ((), ())),
                            preferred_element_type=_F32)
        p = jnp.exp((s - jnp.max(s, axis=-1, keepdims=True)) * scale)
        denom = jnp.sum(p, axis=-1, keepdims=True)
        o = jnp.dot(p.astype(_BF16), kv_buf[slot, 1, g], preferred_element_type=_F32)
        o_scr[hh] = jnp.where(batch_row == i // _HEADS, o / denom, o_scr[hh])
        return carry

    lax.fori_loop(0, n_it, attend, 0)

    w1_sems = [sem.at[_S_W1A]] + [sem.at[_S_W1B]] * (len(_FF_CHUNKS) - 1)
    w2_sems = [sem.at[_S_W2 + k] for k in range(len(_FF_CHUNKS))]
    ff_all = _alternate(ff_copies(w1t_hbm, w1t_v, w1_sems), ff_copies(w2_hbm, w2_v, w2_sems))
    _start(ff_all[:len(ff_all) // 2])

    o_all = jnp.concatenate([o_scr[hh] for hh in range(_HEADS)], axis=-1).astype(_BF16)
    _wait_filled(wo_v, sem.at[_S_O])
    x1 = x + ga * jnp.dot(o_all, wo_v[...], preferred_element_type=_F32)
    h2 = (_layernorm(x1) * (1.0 + cb) + sb).astype(_BF16)
    b2_cp.wait()
    _start(ff_all[len(ff_all) // 2:])

    def hidden(p0, p1, sm):
        _wait_filled(w1t_v.at[pl.ds(p0, p1 - p0)], sm)
        u = lax.dot_general(h2, w1t_v[p0:p1, :], (((1,), (1,)), ((), ())), preferred_element_type=_F32)
        return jax.nn.gelu(u + b1_perm[:, p0:p1], approximate=True).astype(_BF16)

    def project(act, k):
        p0, p1 = ff_pos[k], ff_pos[k + 1]
        _wait_filled(w2_v.at[pl.ds(p0, p1 - p0)], w2_sems[k])
        return jnp.dot(act, w2_v[p0:p1, :], preferred_element_type=_F32)

    y = b2_v[...].astype(_F32).reshape(1, d) + project(hidden(0, ff_pos[1], w1_sems[0]), 0)
    act = hidden(ff_pos[1], ff, w1_sems[1])
    for k in range(1, len(_FF_CHUNKS)):
        y = y + project(act[:, ff_pos[k] - ff_pos[1]:ff_pos[k + 1] - ff_pos[1]], k)
    o_ref[...] = (x1 + gb * y).astype(o_ref.dtype)


@jax.jit
def pallas_adaLN_cond__sliding_block_cached__dense_activation_gelu__decode_kernel(
    A_x: jax.Array,
    A_k_cache: jax.Array,
    A_v_cache: jax.Array,
    A_wq: jax.Array,
    A_wo: jax.Array,
    B_x: jax.Array,
    B_w1: jax.Array,
    B_b1: jax.Array,
    B_w2: jax.Array,
    B_b2: jax.Array,
    c: jax.Array,
    w_mod: jax.Array,
):
    del B_x
    nb, sq, d = A_x.shape
    _, hkv, sk, dh = A_k_cache.shape
    ff = B_w2.shape[0]
    assert sq == 1 and hkv == _HEADS and dh == _DH
    win = min(4096, max(256, sk // 4))
    n_step = nb * hkv // _G

    out = pl.pallas_call(
        _kernel,
        in_specs=[pl.BlockSpec(memory_space=pl.ANY)] * 11,
        out_specs=pl.BlockSpec(memory_space=pltpu.VMEM),
        out_shape=jax.ShapeDtypeStruct((nb, d), A_x.dtype),
        scratch_shapes=[
            pltpu.VMEM((_NBUF, 2, _G, win, dh), _BF16),
            pltpu.VMEM((d, hkv * dh), _BF16),
            pltpu.VMEM((hkv * dh, d), _BF16),
            pltpu.VMEM((ff, d), _BF16),
            pltpu.VMEM((ff, d), _BF16),
            pltpu.VMEM((d, 6 * d), _BF16),
            pltpu.VMEM((nb, d), _BF16),
            pltpu.VMEM((nb, d), _BF16),
            pltpu.VMEM((ff,), _BF16),
            pltpu.VMEM((d,), _BF16),
            pltpu.VMEM((1, ff), _F32),
            pltpu.VMEM((hkv, nb, dh), _BF16),
            pltpu.VMEM((hkv, nb, dh), _F32),
            pltpu.SemaphoreType.DMA((_NSEM,)),
        ],
        compiler_params=pltpu.CompilerParams(
            vmem_limit_bytes=64 * 1024 * 1024,
            disable_bounds_checks=True,
            disable_semaphore_checks=True,
        ),
    )(
        A_x.reshape(nb, d),
        A_k_cache.reshape(n_step, _G, sk, dh),
        A_v_cache.reshape(n_step, _G, sk, dh),
        A_wq, A_wo, B_w1.T, B_b1, B_w2, B_b2, c, w_mod,
    )
    return out.reshape(nb, 1, d)
```

```python
import jax
import jax.numpy as jnp
from jax import lax
import jax.experimental.pallas as pl
import jax.experimental.pallas.tpu as pltpu

_F32 = jnp.float32
_BF16 = jnp.bfloat16
_EPS = 1e-5

_HEADS = 32
_DH = 128
_G = 8
_R = 16
_NBUF = 3
_LOOK = 2
_NSTREAM = 4
_WO_ROWS = 16
_FF_ROWS = 16
_FF_CHUNKS = (288, 96, 48)

_S_KV = 0
_S_C, _S_X, _S_B1, _S_B2, _S_MOD, _S_Q, _S_O, _S_W1A, _S_W1B, _S_W2 = range(_NBUF, _NBUF + 10)
_NSEM = _S_W2 + len(_FF_CHUNKS)


def _layernorm(x):
    m = jnp.mean(x, axis=-1, keepdims=True)
    xc = x - m
    v = jnp.mean(xc * xc, axis=-1, keepdims=True)
    return xc * lax.rsqrt(v + _EPS)


def _alternate(a, b):
    assert len(a) == len(b)
    return [t for x, y in zip(a, b) for t in (x + (0,), y + (1,))]


def _streamed(src, dst, sem, cols):
    nrows, ncols = src.shape
    n = nrows // (2 * _NSTREAM)
    queues = ([], [])
    for j in range(n // 8):
        for c in range(0, ncols, cols(j)):
            for s in range(2 * _NSTREAM):
                idx = (pl.ds(s * n + j * 8, 8), pl.ds(c, cols(j)))
                queues[s // _NSTREAM].append((src.at[idx], dst.at[idx], sem))
    return _alternate(*queues)


def _start(copies):
    for src, dst, sem, queue in copies:
        pltpu.make_async_copy(src, dst, sem).start(priority=queue)


def _wait_filled(view, sem):
    pltpu.make_async_copy(view, view, sem).wait()


def _kernel(x_hbm, k_hbm, v_hbm, wq_hbm, wo_hbm, w1t_hbm, b1_hbm, w2_hbm, b2_hbm, c_hbm, wmod_hbm,
            o_ref,
            kv_buf, wq_v, wo_v, w1t_v, w2_v, wmod_v, x_v, c_v, b1_v, b2_v, b1_perm, q_scr, o_scr, sem):
    nb, d = x_v.shape
    ff = w2_v.shape[0]
    win = kv_buf.shape[3]
    row0 = k_hbm.shape[2] - win
    n_desc = win // _R
    per_it = n_desc // _G
    n_it = nb * _HEADS
    n_tail = _LOOK * _G
    scale = _DH ** -0.5

    def start_kv(step, slot, r_first, n):
        for j in range(n):
            r = r_first + j * _R
            if not isinstance(r, int):
                r = pl.multiple_of(r, _R)
            for which, src in enumerate((k_hbm, v_hbm)):
                pltpu.make_async_copy(src.at[step, :, pl.ds(row0 + r, _R), :],
                                      kv_buf.at[slot, which, :, pl.ds(r, _R), :],
                                      sem.at[_S_KV + slot]).start(priority=1 - which)

    ff_stream = ff // _NSTREAM
    assert sum(_FF_CHUNKS) == ff_stream
    ff_pos = [_NSTREAM * sum(_FF_CHUNKS[:k]) for k in range(len(_FF_CHUNKS) + 1)]

    def ff_rows(k, s):
        return s * ff_stream + sum(_FF_CHUNKS[:k]), ff_pos[k] + s * _FF_CHUNKS[k]

    def ff_copies(src, dst, sems):
        out = []
        for k, n in enumerate(_FF_CHUNKS):
            for j in range(0, n, _FF_ROWS):
                for s in range(_NSTREAM):
                    r_src, r_dst = ff_rows(k, s)
                    out.append((src.at[pl.ds(r_src + j, _FF_ROWS), :], dst.at[pl.ds(r_dst + j, _FF_ROWS), :],
                                sems[k]))
        return out

    c_cp = pltpu.make_async_copy(c_hbm, c_v, sem.at[_S_C])
    x_cp = pltpu.make_async_copy(x_hbm, x_v, sem.at[_S_X])
    b1_cp = pltpu.make_async_copy(b1_hbm, b1_v, sem.at[_S_B1])
    b2_cp = pltpu.make_async_copy(b2_hbm, b2_v, sem.at[_S_B2])

    _start(_streamed(wmod_hbm, wmod_v, sem.at[_S_MOD], lambda j: d if j < 2 else 3 * d))
    for cp in (c_cp, x_cp, b1_cp, b2_cp):
        cp.start()
    _start(_streamed(wq_hbm, wq_v, sem.at[_S_Q], lambda j: _HEADS * _DH // 2))

    c_cp.wait()
    x_cp.wait()
    b1_cp.wait()
    _wait_filled(wmod_v, sem.at[_S_MOD])
    b1 = b1_v[...].astype(_F32).reshape(1, ff)
    for k, n in enumerate(_FF_CHUNKS):
        for s in range(_NSTREAM):
            r_src, r_dst = ff_rows(k, s)
            b1_perm[:, r_dst:r_dst + n] = b1[:, r_src:r_src + n]
    c = c_v[...].astype(_F32)
    mod = jnp.dot((c * jax.nn.sigmoid(c)).astype(_BF16), wmod_v[...], preferred_element_type=_F32)
    sa, ca, ga, sb, cb, gb = (mod[:, k * d:(k + 1) * d] for k in range(6))
    x = x_v[...].astype(_F32)
    h = (_layernorm(x) * (1.0 + ca) + sa).astype(_BF16)

    start_kv(0, 0, 0, n_desc // 2)
    _wait_filled(wq_v, sem.at[_S_Q])
    q = jnp.dot(h, wq_v[...], preferred_element_type=_F32)
    for hh in range(_HEADS):
        q_scr[hh] = q[:, hh * _DH:(hh + 1) * _DH].astype(_BF16)
    o_scr[...] = jnp.zeros_like(o_scr)
    start_kv(0, 0, (n_desc // 2) * _R, n_desc // 2)
    for s in range(1, _LOOK):
        start_kv(s, s, 0, n_desc)

    batch_row = lax.broadcasted_iota(jnp.int32, (nb, _DH), 0)
    wo_half = _HEADS * _DH // 2
    wo_stream = wo_half // _NSTREAM
    wo_per_it = wo_stream // n_tail

    def attend(i, carry):
        step = i // _G
        g = i % _G
        slot = step % _NBUF

        @pl.when(i < n_it - n_tail)
        def _():
            start_kv(step + _LOOK, (step + _LOOK) % _NBUF, g * (per_it * _R), per_it)

        @pl.when(i >= n_it - n_tail)
        def _():
            t = i - (n_it - n_tail)
            for j in range(0, wo_per_it, _WO_ROWS):
                for s in range(_NSTREAM):
                    for queue in range(2):
                        r = queue * wo_half + s * wo_stream + t * wo_per_it + j
                        rows = pl.ds(pl.multiple_of(r, _WO_ROWS), _WO_ROWS)
                        pltpu.make_async_copy(wo_hbm.at[rows, :], wo_v.at[rows, :],
                                              sem.at[_S_O]).start(priority=queue)

        @pl.when(g == 0)
        def _():
            _wait_filled(kv_buf.at[slot], sem.at[_S_KV + slot])

        hh = i % _HEADS
        s = lax.dot_general(q_scr[hh], kv_buf[slot, 0, g], (((1,), (1,)), ((), ())),
                            preferred_element_type=_F32)
        p = jnp.exp((s - jnp.max(s, axis=-1, keepdims=True)) * scale)
        denom = jnp.sum(p, axis=-1, keepdims=True)
        o = jnp.dot(p.astype(_BF16), kv_buf[slot, 1, g], preferred_element_type=_F32)
        o_scr[hh] = jnp.where(batch_row == i // _HEADS, o / denom, o_scr[hh])
        return carry

    lax.fori_loop(0, n_it, attend, 0)

    w1_sems = [sem.at[_S_W1A]] + [sem.at[_S_W1B]] * (len(_FF_CHUNKS) - 1)
    w2_sems = [sem.at[_S_W2 + k] for k in range(len(_FF_CHUNKS))]
    ff_all = _alternate(ff_copies(w1t_hbm, w1t_v, w1_sems), ff_copies(w2_hbm, w2_v, w2_sems))
    _start(ff_all[:len(ff_all) // 2])

    o_all = jnp.concatenate([o_scr[hh] for hh in range(_HEADS)], axis=-1).astype(_BF16)
    _wait_filled(wo_v, sem.at[_S_O])
    x1 = x + ga * jnp.dot(o_all, wo_v[...], preferred_element_type=_F32)
    h2 = (_layernorm(x1) * (1.0 + cb) + sb).astype(_BF16)
    b2_cp.wait()
    _start(ff_all[len(ff_all) // 2:])

    def hidden(p0, p1, sm):
        _wait_filled(w1t_v.at[pl.ds(p0, p1 - p0)], sm)
        u = lax.dot_general(h2, w1t_v[p0:p1, :], (((1,), (1,)), ((), ())), preferred_element_type=_F32)
        return jax.nn.gelu(u + b1_perm[:, p0:p1], approximate=True).astype(_BF16)

    def project(act, k):
        p0, p1 = ff_pos[k], ff_pos[k + 1]
        _wait_filled(w2_v.at[pl.ds(p0, p1 - p0)], w2_sems[k])
        return jnp.dot(act, w2_v[p0:p1, :], preferred_element_type=_F32)

    y = b2_v[...].astype(_F32).reshape(1, d) + project(hidden(0, ff_pos[1], w1_sems[0]), 0)
    act = hidden(ff_pos[1], ff, w1_sems[1])
    for k in range(1, len(_FF_CHUNKS)):
        y = y + project(act[:, ff_pos[k] - ff_pos[1]:ff_pos[k + 1] - ff_pos[1]], k)
    o_ref[...] = (x1 + gb * y).astype(o_ref.dtype)


@jax.jit
def pallas_adaLN_cond__sliding_block_cached__dense_activation_gelu__decode_kernel(
    A_x: jax.Array,
    A_k_cache: jax.Array,
    A_v_cache: jax.Array,
    A_wq: jax.Array,
    A_wo: jax.Array,
    B_x: jax.Array,
    B_w1: jax.Array,
    B_b1: jax.Array,
    B_w2: jax.Array,
    B_b2: jax.Array,
    c: jax.Array,
    w_mod: jax.Array,
):
    del B_x
    nb, sq, d = A_x.shape
    _, hkv, sk, dh = A_k_cache.shape
    ff = B_w2.shape[0]
    assert sq == 1 and hkv == _HEADS and dh == _DH
    win = min(4096, max(256, sk // 4))
    n_step = nb * hkv // _G

    out = pl.pallas_call(
        _kernel,
        in_specs=[pl.BlockSpec(memory_space=pl.ANY)] * 11,
        out_specs=pl.BlockSpec(memory_space=pltpu.VMEM),
        out_shape=jax.ShapeDtypeStruct((nb, d), A_x.dtype),
        scratch_shapes=[
            pltpu.VMEM((_NBUF, 2, _G, win, dh), _BF16),
            pltpu.VMEM((d, hkv * dh), _BF16),
            pltpu.VMEM((hkv * dh, d), _BF16),
            pltpu.VMEM((ff, d), _BF16),
            pltpu.VMEM((ff, d), _BF16),
            pltpu.VMEM((d, 6 * d), _BF16),
            pltpu.VMEM((nb, d), _BF16),
            pltpu.VMEM((nb, d), _BF16),
            pltpu.VMEM((ff,), _BF16),
            pltpu.VMEM((d,), _BF16),
            pltpu.VMEM((1, ff), _F32),
            pltpu.VMEM((hkv, nb, dh), _BF16),
            pltpu.VMEM((hkv, nb, dh), _F32),
            pltpu.SemaphoreType.DMA((_NSEM,)),
        ],
        compiler_params=pltpu.CompilerParams(
            vmem_limit_bytes=64 * 1024 * 1024,
            disable_bounds_checks=True,
            disable_semaphore_checks=True,
        ),
    )(
        A_x.reshape(nb, d),
        A_k_cache.reshape(n_step, _G, sk, dh),
        A_v_cache.reshape(n_step, _G, sk, dh),
        A_wq, A_wo, B_w1.T, B_b1, B_w2, B_b2, c, w_mod,
    )
    return out.reshape(nb, 1, d)
```

```python
import jax
import jax.numpy as jnp
from jax import lax
import jax.experimental.pallas as pl
import jax.experimental.pallas.tpu as pltpu

_F32 = jnp.float32
_BF16 = jnp.bfloat16
_EPS = 1e-5

_HEADS = 32
_DH = 128
_NSTREAM = 4
_G = _NSTREAM
_NBUF = 3
_LOOK = 2
_KV_ROWS = 128
_BLOCK = 16
_WMOD_SKEW = 8
_FF_ROWS = 16
_FF_CHUNKS = (288, 96, 48)

_S_KV = 0
_S_C, _S_X, _S_B1, _S_B2, _S_MOD, _S_Q, _S_O, _S_W1A, _S_W1B, _S_W2 = range(_NBUF, _NBUF + 10)
_NSEM = _S_W2 + len(_FF_CHUNKS)


def _layernorm(x):
    m = jnp.mean(x, axis=-1, keepdims=True)
    xc = x - m
    v = jnp.mean(xc * xc, axis=-1, keepdims=True)
    return xc * lax.rsqrt(v + _EPS)


def _bursts(t0, t1, width, skew=0, block=_BLOCK):
    out = []
    while t0 < t1:
        end = min(t1, ((t0 + skew) // block + 1) * block - skew)
        rects = []
        while t0 < end:
            r, c = divmod(t0, width)
            nr, nc = ((end - t0) // width, width) if c == 0 and end - t0 >= width else (1, min(width - c, end - t0))
            rects.append((8 * r, 8 * nr, 128 * c, 128 * nc))
            t0 += nr * nc
        out.append(rects)
    return out


def _whole_array(src, dst, sem, skew=0, fine=0):
    width = src.shape[1] // 128
    n_tiles = src.shape[0] // 8 * width
    cuts = [0] + list(range(_BLOCK - skew if skew else _BLOCK, n_tiles, _BLOCK)) + [n_tiles]
    first = [(len(cuts) - 1) * s // (2 * _NSTREAM) for s in range(2 * _NSTREAM + 1)]
    streams = [_bursts(cuts[a], cuts[a + fine], width, skew, _BLOCK // 4) + _bursts(cuts[a + fine], cuts[b], width, skew)
               for a, b in zip(first[:-1], first[1:])]
    queues = [[st[i] for i in range(max(map(len, half))) for st in half if i < len(st)]
              for half in (streams[:_NSTREAM], streams[_NSTREAM:])]
    out = []
    for i in range(max(map(len, queues))):
        for queue in range(2):
            for r, nr, c, nc in queues[queue][i] if i < len(queues[queue]) else ():
                idx = (pl.ds(r, nr), pl.ds(c, nc))
                out.append((src.at[idx], dst.at[idx], sem, queue))
    return out


def _start(copies):
    for src, dst, sem, queue in copies:
        pltpu.make_async_copy(src, dst, sem).start(priority=queue)


def _wait_filled(view, sem):
    pltpu.make_async_copy(view, view, sem).wait()


def _kernel(x_hbm, k_hbm, v_hbm, wq_hbm, wo_hbm, w1t_hbm, b1_hbm, w2_hbm, b2_hbm, c_hbm, wmod_hbm,
            o_ref,
            kv_buf, wq_v, wo_v, w1t_v, w2_v, wmod_v, x_v, c_v, b1_v, b2_v, b1_perm, q_scr, o_scr, sem):
    nb, d = x_v.shape
    ff = w2_v.shape[0]
    win = kv_buf.shape[3]
    row0 = k_hbm.shape[2] - win
    n_it = nb * _HEADS
    n_tail = _LOOK * _G
    scale = _DH ** -0.5

    def start_kv(step, slot, r_first, n_rows):
        for j in range(0, n_rows, _KV_ROWS):
            r = r_first + j
            if not isinstance(r, int):
                r = pl.multiple_of(r, _KV_ROWS)
            for g in range(_G):
                for which, src in enumerate((k_hbm, v_hbm)):
                    pltpu.make_async_copy(src.at[step, g, pl.ds(row0 + r, _KV_ROWS), :],
                                          kv_buf.at[slot, which, g, pl.ds(r, _KV_ROWS), :],
                                          sem.at[_S_KV + slot]).start(priority=1 - which)

    ff_stream = ff // _NSTREAM
    assert sum(_FF_CHUNKS) == ff_stream
    ff_pos = [_NSTREAM * sum(_FF_CHUNKS[:k]) for k in range(len(_FF_CHUNKS) + 1)]

    def ff_rows(k, s):
        return s * ff_stream + sum(_FF_CHUNKS[:k]), ff_pos[k] + s * _FF_CHUNKS[k]

    c_cp = pltpu.make_async_copy(c_hbm, c_v, sem.at[_S_C])
    x_cp = pltpu.make_async_copy(x_hbm, x_v, sem.at[_S_X])
    b1_cp = pltpu.make_async_copy(b1_hbm, b1_v, sem.at[_S_B1])
    b2_cp = pltpu.make_async_copy(b2_hbm, b2_v, sem.at[_S_B2])

    _start(_whole_array(wmod_hbm, wmod_v, sem.at[_S_MOD], skew=_WMOD_SKEW, fine=2))
    for cp in (c_cp, x_cp, b1_cp, b2_cp):
        cp.start()
    _start(_whole_array(wq_hbm, wq_v, sem.at[_S_Q]))

    c_cp.wait()
    x_cp.wait()
    b1_cp.wait()
    _wait_filled(wmod_v, sem.at[_S_MOD])
    b1 = b1_v[...].astype(_F32).reshape(1, ff)
    for k, n in enumerate(_FF_CHUNKS):
        for s in range(_NSTREAM):
            r_src, r_dst = ff_rows(k, s)
            b1_perm[:, r_dst:r_dst + n] = b1[:, r_src:r_src + n]
    c = c_v[...].astype(_F32)
    mod = jnp.dot((c * jax.nn.sigmoid(c)).astype(_BF16), wmod_v[...], preferred_element_type=_F32)
    sa, ca, ga, sb, cb, gb = (mod[:, k * d:(k + 1) * d] for k in range(6))
    x = x_v[...].astype(_F32)
    h = (_layernorm(x) * (1.0 + ca) + sa).astype(_BF16)

    start_kv(0, 0, 0, win)
    _wait_filled(wq_v, sem.at[_S_Q])
    q = jnp.dot(h, wq_v[...], preferred_element_type=_F32)
    for hh in range(_HEADS):
        q_scr[hh] = q[:, hh * _DH:(hh + 1) * _DH].astype(_BF16)
    o_scr[...] = jnp.zeros_like(o_scr)
    for s in range(1, _LOOK):
        start_kv(s, s, 0, win)

    batch_row = lax.broadcasted_iota(jnp.int32, (nb, _DH), 0)
    wo_stream = _HEADS * _DH // (2 * _NSTREAM)
    wo_period = _bursts(0, _BLOCK * (d // 128), d // 128)
    wo_parts = n_tail * 8 * _BLOCK // wo_stream
    wo_cuts = [-(-len(wo_period) * k // wo_parts) for k in range(wo_parts + 1)]

    def attend(i, carry):
        step = i // _G
        g = i % _G
        slot = step % _NBUF
        t = i - (n_it - n_tail)

        @pl.when(t < 0)
        def _():
            start_kv(step + _LOOK, (step + _LOOK) % _NBUF, g * (win // _G), win // _G)

        for part in range(wo_parts):
            @pl.when(jnp.logical_and(t >= 0, t % wo_parts == part))
            def _():
                base = (t // wo_parts) * (8 * _BLOCK)
                for rects in wo_period[wo_cuts[part]:wo_cuts[part + 1]]:
                    for s in range(_NSTREAM):
                        for queue in range(2):
                            for r, nr, c0, nc in rects:
                                r = pl.multiple_of((queue * _NSTREAM + s) * wo_stream + base + r, 8)
                                idx = (pl.ds(r, nr), pl.ds(c0, nc))
                                pltpu.make_async_copy(wo_hbm.at[idx], wo_v.at[idx],
                                                      sem.at[_S_O]).start(priority=queue)

        @pl.when(g == 0)
        def _():
            _wait_filled(kv_buf.at[slot], sem.at[_S_KV + slot])

        hh = i % _HEADS
        s = lax.dot_general(q_scr[hh], kv_buf[slot, 0, g], (((1,), (1,)), ((), ())),
                            preferred_element_type=_F32)
        p = jnp.exp((s - jnp.max(s, axis=-1, keepdims=True)) * scale)
        denom = jnp.sum(p, axis=-1, keepdims=True)
        o = jnp.dot(p.astype(_BF16), kv_buf[slot, 1, g], preferred_element_type=_F32)
        o_scr[hh] = jnp.where(batch_row == i // _HEADS, o / denom, o_scr[hh])
        return carry

    lax.fori_loop(0, n_it, attend, 0)

    w1_sems = [sem.at[_S_W1A]] + [sem.at[_S_W1B]] * (len(_FF_CHUNKS) - 1)
    w2_sems = [sem.at[_S_W2 + k] for k in range(len(_FF_CHUNKS))]
    ff_copies = []
    for k, n in enumerate(_FF_CHUNKS):
        for j in range(0, n, _FF_ROWS):
            for s in range(_NSTREAM):
                r_src, r_dst = (pl.ds(r + j, _FF_ROWS) for r in ff_rows(k, s))
                ff_copies.append((w1t_hbm.at[r_src, :], w1t_v.at[r_dst, :], w1_sems[k], 0))
                ff_copies.append((w2_hbm.at[r_src, :], w2_v.at[r_dst, :], w2_sems[k], 1))
    _start(ff_copies[:len(ff_copies) // 2])

    o_all = jnp.concatenate([o_scr[hh] for hh in range(_HEADS)], axis=-1).astype(_BF16)
    _wait_filled(wo_v, sem.at[_S_O])
    x1 = x + ga * jnp.dot(o_all, wo_v[...], preferred_element_type=_F32)
    h2 = (_layernorm(x1) * (1.0 + cb) + sb).astype(_BF16)
    b2_cp.wait()
    _start(ff_copies[len(ff_copies) // 2:])

    def hidden(p0, p1, sm):
        _wait_filled(w1t_v.at[pl.ds(p0, p1 - p0)], sm)
        u = lax.dot_general(h2, w1t_v[p0:p1, :], (((1,), (1,)), ((), ())), preferred_element_type=_F32)
        return jax.nn.gelu(u + b1_perm[:, p0:p1], approximate=True).astype(_BF16)

    def project(act, k):
        p0, p1 = ff_pos[k], ff_pos[k + 1]
        _wait_filled(w2_v.at[pl.ds(p0, p1 - p0)], w2_sems[k])
        return jnp.dot(act, w2_v[p0:p1, :], preferred_element_type=_F32)

    y = b2_v[...].astype(_F32).reshape(1, d) + project(hidden(0, ff_pos[1], w1_sems[0]), 0)
    act = hidden(ff_pos[1], ff, w1_sems[1])
    for k in range(1, len(_FF_CHUNKS)):
        y = y + project(act[:, ff_pos[k] - ff_pos[1]:ff_pos[k + 1] - ff_pos[1]], k)
    o_ref[...] = (x1 + gb * y).astype(o_ref.dtype)


@jax.jit
def pallas_adaLN_cond__sliding_block_cached__dense_activation_gelu__decode_kernel(
    A_x: jax.Array,
    A_k_cache: jax.Array,
    A_v_cache: jax.Array,
    A_wq: jax.Array,
    A_wo: jax.Array,
    B_x: jax.Array,
    B_w1: jax.Array,
    B_b1: jax.Array,
    B_w2: jax.Array,
    B_b2: jax.Array,
    c: jax.Array,
    w_mod: jax.Array,
):
    del B_x
    nb, sq, d = A_x.shape
    _, hkv, sk, dh = A_k_cache.shape
    ff = B_w2.shape[0]
    assert sq == 1 and hkv == _HEADS and dh == _DH
    win = min(4096, max(256, sk // 4))
    assert win % (_G * _KV_ROWS) == 0
    n_step = nb * hkv // _G

    out = pl.pallas_call(
        _kernel,
        in_specs=[pl.BlockSpec(memory_space=pl.ANY)] * 11,
        out_specs=pl.BlockSpec(memory_space=pltpu.VMEM),
        out_shape=jax.ShapeDtypeStruct((nb, d), A_x.dtype),
        scratch_shapes=[
            pltpu.VMEM((_NBUF, 2, _G, win, dh), _BF16),
            pltpu.VMEM((d, hkv * dh), _BF16),
            pltpu.VMEM((hkv * dh, d), _BF16),
            pltpu.VMEM((ff, d), _BF16),
            pltpu.VMEM((ff, d), _BF16),
            pltpu.VMEM((d, 6 * d), _BF16),
            pltpu.VMEM((nb, d), _BF16),
            pltpu.VMEM((nb, d), _BF16),
            pltpu.VMEM((ff,), _BF16),
            pltpu.VMEM((d,), _BF16),
            pltpu.VMEM((1, ff), _F32),
            pltpu.VMEM((hkv, nb, dh), _BF16),
            pltpu.VMEM((hkv, nb, dh), _F32),
            pltpu.SemaphoreType.DMA((_NSEM,)),
        ],
        compiler_params=pltpu.CompilerParams(
            vmem_limit_bytes=48 * 1024 * 1024,
            disable_bounds_checks=True,
            disable_semaphore_checks=True,
        ),
    )(
        A_x.reshape(nb, d),
        A_k_cache.reshape(n_step, _G, sk, dh),
        A_v_cache.reshape(n_step, _G, sk, dh),
        A_wq, A_wo, B_w1.T, B_b1, B_w2, B_b2, c, w_mod,
    )
    return out.reshape(nb, 1, d)
```

```python
import jax
import jax.numpy as jnp
from jax import lax
import jax.experimental.pallas as pl
import jax.experimental.pallas.tpu as pltpu

_F32 = jnp.float32
_BF16 = jnp.bfloat16
_EPS = 1e-5

_HEADS = 32
_DH = 128
_NSTREAM = 4
_G = _NSTREAM
_NBUF = 3
_LOOK = 2
_BLOCK = 16
_KV_ROWS = 8 * _BLOCK
_KV_SKEW = 4
_WMOD_SKEW = 8
_FF_ROWS = 16
_FF_CHUNKS = (288, 96, 48)

_S_KV, _S_EDGE = 0, _NBUF
_S_C, _S_X, _S_B1, _S_B2, _S_MOD, _S_Q, _S_O, _S_W1A, _S_W1B, _S_W2 = range(2 * _NBUF, 2 * _NBUF + 10)
_NSEM = _S_W2 + len(_FF_CHUNKS)


def _layernorm(x):
    m = jnp.mean(x, axis=-1, keepdims=True)
    xc = x - m
    v = jnp.mean(xc * xc, axis=-1, keepdims=True)
    return xc * lax.rsqrt(v + _EPS)


def _bursts(t0, t1, width, skew=0, block=_BLOCK):
    out = []
    while t0 < t1:
        end = min(t1, ((t0 + skew) // block + 1) * block - skew)
        rects = []
        while t0 < end:
            r, c = divmod(t0, width)
            nr, nc = ((end - t0) // width, width) if c == 0 and end - t0 >= width else (1, min(width - c, end - t0))
            rects.append((8 * r, 8 * nr, 128 * c, 128 * nc))
            t0 += nr * nc
        out.append(rects)
    return out


def _whole_array(src, dst, sem, skew=0, fine=0):
    width = src.shape[1] // 128
    n_tiles = src.shape[0] // 8 * width
    cuts = [0] + list(range(_BLOCK - skew if skew else _BLOCK, n_tiles, _BLOCK)) + [n_tiles]
    first = [(len(cuts) - 1) * s // (2 * _NSTREAM) for s in range(2 * _NSTREAM + 1)]
    streams = [_bursts(cuts[a], cuts[a + fine], width, skew, _BLOCK // 4) + _bursts(cuts[a + fine], cuts[b], width, skew)
               for a, b in zip(first[:-1], first[1:])]
    queues = [[st[i] for i in range(max(map(len, half))) for st in half if i < len(st)]
              for half in (streams[:_NSTREAM], streams[_NSTREAM:])]
    out = []
    for i in range(max(map(len, queues))):
        for queue in range(2):
            for r, nr, c, nc in queues[queue][i] if i < len(queues[queue]) else ():
                idx = (pl.ds(r, nr), pl.ds(c, nc))
                out.append((src.at[idx], dst.at[idx], sem, queue))
    return out


def _start(copies):
    for src, dst, sem, queue in copies:
        pltpu.make_async_copy(src, dst, sem).start(priority=queue)


def _wait_filled(view, sem):
    pltpu.make_async_copy(view, view, sem).wait()


def _kernel(x_hbm, k_hbm, v_hbm, k4_hbm, v4_hbm, wq_hbm, wo_hbm, w1t_hbm, b1_hbm, w2_hbm, b2_hbm, c_hbm, wmod_hbm,
            o_ref,
            kv_buf, edge_buf, wq_v, wo_v, w1t_v, w2_v, wmod_v, x_v, c_v, b1_v, b2_v, b1_perm, q_scr, o_scr, sem):
    nb, d = x_v.shape
    ff = w2_v.shape[0]
    n_edge = edge_buf.shape[3]
    n_blk = n_edge // 2
    win = n_blk * _KV_ROWS
    row0 = k_hbm.shape[2] - win
    n_it = nb * _HEADS
    n_tail = _LOOK * _G
    scale = _DH ** -0.5

    def start_kv(step, slot, j_first, n):
        body = _KV_ROWS - 2 * _KV_SKEW
        for jj in range(n):
            j = j_first + jj
            hint = (lambda v, m: v) if isinstance(j, int) else pl.multiple_of
            e_lead, e_trail = (2 * j + n_edge - 1) % n_edge, 2 * j
            for g in range(_G):
                for which, (src, src4) in enumerate(((k_hbm, k4_hbm), (v_hbm, v4_hbm))):
                    def edge(e):
                        unit = (row0 + (e // 2) * _KV_ROWS + body) // _KV_SKEW + e % 2
                        return (src4.at[step, g, pl.ds(unit, 1)], edge_buf.at[slot, which, g, pl.ds(e, 1)],
                                sem.at[_S_EDGE + slot], 1 - which)
                    _start([edge(e_lead),
                            (src.at[step, g, pl.ds(hint(row0 + j * _KV_ROWS, _KV_ROWS), body), :],
                             kv_buf.at[slot, which, g, pl.ds(hint(j * body, 8), body), :],
                             sem.at[_S_KV + slot], 1 - which),
                            edge(e_trail)])

    ff_stream = ff // _NSTREAM
    assert sum(_FF_CHUNKS) == ff_stream
    ff_pos = [_NSTREAM * sum(_FF_CHUNKS[:k]) for k in range(len(_FF_CHUNKS) + 1)]

    def ff_rows(k, s):
        return s * ff_stream + sum(_FF_CHUNKS[:k]), ff_pos[k] + s * _FF_CHUNKS[k]

    c_cp = pltpu.make_async_copy(c_hbm, c_v, sem.at[_S_C])
    x_cp = pltpu.make_async_copy(x_hbm, x_v, sem.at[_S_X])
    b1_cp = pltpu.make_async_copy(b1_hbm, b1_v, sem.at[_S_B1])
    b2_cp = pltpu.make_async_copy(b2_hbm, b2_v, sem.at[_S_B2])

    _start(_whole_array(wmod_hbm, wmod_v, sem.at[_S_MOD], skew=_WMOD_SKEW, fine=2))
    for cp in (c_cp, x_cp, b1_cp, b2_cp):
        cp.start()
    _start(_whole_array(wq_hbm, wq_v, sem.at[_S_Q]))

    c_cp.wait()
    x_cp.wait()
    b1_cp.wait()
    _wait_filled(wmod_v, sem.at[_S_MOD])
    b1 = b1_v[...].astype(_F32).reshape(1, ff)
    for k, n in enumerate(_FF_CHUNKS):
        for s in range(_NSTREAM):
            r_src, r_dst = ff_rows(k, s)
            b1_perm[:, r_dst:r_dst + n] = b1[:, r_src:r_src + n]
    c = c_v[...].astype(_F32)
    mod = jnp.dot((c * jax.nn.sigmoid(c)).astype(_BF16), wmod_v[...], preferred_element_type=_F32)
    sa, ca, ga, sb, cb, gb = (mod[:, k * d:(k + 1) * d] for k in range(6))
    x = x_v[...].astype(_F32)
    h = (_layernorm(x) * (1.0 + ca) + sa).astype(_BF16)

    start_kv(0, 0, 0, n_blk)
    _wait_filled(wq_v, sem.at[_S_Q])
    q = jnp.dot(h, wq_v[...], preferred_element_type=_F32)
    for hh in range(_HEADS):
        q_scr[hh] = q[:, hh * _DH:(hh + 1) * _DH].astype(_BF16)
    o_scr[...] = jnp.zeros_like(o_scr)
    for s in range(1, _LOOK):
        start_kv(s, s, 0, n_blk)

    batch_row = lax.broadcasted_iota(jnp.int32, (nb, _DH), 0)
    wo_stream = _HEADS * _DH // (2 * _NSTREAM)
    wo_period = _bursts(0, _BLOCK * (d // 128), d // 128)
    wo_parts = n_tail * 8 * _BLOCK // wo_stream
    wo_cuts = [-(-len(wo_period) * k // wo_parts) for k in range(wo_parts + 1)]

    def attend(i, carry):
        step = i // _G
        g = i % _G
        slot = step % _NBUF
        t = i - (n_it - n_tail)

        @pl.when(t < 0)
        def _():
            start_kv(step + _LOOK, (step + _LOOK) % _NBUF, g * (n_blk // _G), n_blk // _G)

        for part in range(wo_parts):
            @pl.when(jnp.logical_and(t >= 0, t % wo_parts == part))
            def _():
                base = (t // wo_parts) * (8 * _BLOCK)
                for rects in wo_period[wo_cuts[part]:wo_cuts[part + 1]]:
                    for s in range(_NSTREAM):
                        for queue in range(2):
                            for r, nr, c0, nc in rects:
                                r = pl.multiple_of((queue * _NSTREAM + s) * wo_stream + base + r, 8)
                                idx = (pl.ds(r, nr), pl.ds(c0, nc))
                                pltpu.make_async_copy(wo_hbm.at[idx], wo_v.at[idx],
                                                      sem.at[_S_O]).start(priority=queue)

        @pl.when(g == 0)
        def _():
            _wait_filled(kv_buf.at[slot], sem.at[_S_KV + slot])
            _wait_filled(edge_buf.at[slot], sem.at[_S_EDGE + slot])

        hh = i % _HEADS
        k_edge, v_edge = (edge_buf[slot, which, g].reshape(n_edge * _KV_SKEW, _DH) for which in range(2))
        s = jnp.concatenate(
            [lax.dot_general(q_scr[hh], k, (((1,), (1,)), ((), ())), preferred_element_type=_F32)
             for k in (kv_buf[slot, 0, g], k_edge)], axis=-1)
        p = jnp.exp((s - jnp.max(s, axis=-1, keepdims=True)) * scale)
        denom = jnp.sum(p, axis=-1, keepdims=True)
        p = p.astype(_BF16)
        n_body = kv_buf.shape[3]
        o = (jnp.dot(p[:, :n_body], kv_buf[slot, 1, g], preferred_element_type=_F32)
             + jnp.dot(p[:, n_body:], v_edge, preferred_element_type=_F32))
        o_scr[hh] = jnp.where(batch_row == i // _HEADS, o / denom, o_scr[hh])
        return carry

    lax.fori_loop(0, n_it, attend, 0)

    w1_sems = [sem.at[_S_W1A]] + [sem.at[_S_W1B]] * (len(_FF_CHUNKS) - 1)
    w2_sems = [sem.at[_S_W2 + k] for k in range(len(_FF_CHUNKS))]
    ff_copies = []
    for k, n in enumerate(_FF_CHUNKS):
        for j in range(0, n, _FF_ROWS):
            for s in range(_NSTREAM):
                r_src, r_dst = (pl.ds(r + j, _FF_ROWS) for r in ff_rows(k, s))
                ff_copies.append((w1t_hbm.at[r_src, :], w1t_v.at[r_dst, :], w1_sems[k], 0))
                ff_copies.append((w2_hbm.at[r_src, :], w2_v.at[r_dst, :], w2_sems[k], 1))
    _start(ff_copies[:len(ff_copies) // 2])

    o_all = jnp.concatenate([o_scr[hh] for hh in range(_HEADS)], axis=-1).astype(_BF16)
    _wait_filled(wo_v, sem.at[_S_O])
    x1 = x + ga * jnp.dot(o_all, wo_v[...], preferred_element_type=_F32)
    h2 = (_layernorm(x1) * (1.0 + cb) + sb).astype(_BF16)
    b2_cp.wait()
    _start(ff_copies[len(ff_copies) // 2:])

    def hidden(p0, p1, sm):
        _wait_filled(w1t_v.at[pl.ds(p0, p1 - p0)], sm)
        u = lax.dot_general(h2, w1t_v[p0:p1, :], (((1,), (1,)), ((), ())), preferred_element_type=_F32)
        return jax.nn.gelu(u + b1_perm[:, p0:p1], approximate=True).astype(_BF16)

    def project(act, k):
        p0, p1 = ff_pos[k], ff_pos[k + 1]
        _wait_filled(w2_v.at[pl.ds(p0, p1 - p0)], w2_sems[k])
        return jnp.dot(act, w2_v[p0:p1, :], preferred_element_type=_F32)

    y = b2_v[...].astype(_F32).reshape(1, d) + project(hidden(0, ff_pos[1], w1_sems[0]), 0)
    act = hidden(ff_pos[1], ff, w1_sems[1])
    for k in range(1, len(_FF_CHUNKS)):
        y = y + project(act[:, ff_pos[k] - ff_pos[1]:ff_pos[k + 1] - ff_pos[1]], k)
    o_ref[...] = (x1 + gb * y).astype(o_ref.dtype)


@jax.jit
def pallas_adaLN_cond__sliding_block_cached__dense_activation_gelu__decode_kernel(
    A_x: jax.Array,
    A_k_cache: jax.Array,
    A_v_cache: jax.Array,
    A_wq: jax.Array,
    A_wo: jax.Array,
    B_x: jax.Array,
    B_w1: jax.Array,
    B_b1: jax.Array,
    B_w2: jax.Array,
    B_b2: jax.Array,
    c: jax.Array,
    w_mod: jax.Array,
):
    del B_x
    nb, sq, d = A_x.shape
    _, hkv, sk, dh = A_k_cache.shape
    ff = B_w2.shape[0]
    assert sq == 1 and hkv == _HEADS and dh == _DH
    win = min(4096, max(256, sk // 4))
    assert win % (_G * _KV_ROWS) == 0
    n_blk = win // _KV_ROWS
    n_step = nb * hkv // _G

    out = pl.pallas_call(
        _kernel,
        in_specs=[pl.BlockSpec(memory_space=pl.ANY)] * 13,
        out_specs=pl.BlockSpec(memory_space=pltpu.VMEM),
        out_shape=jax.ShapeDtypeStruct((nb, d), A_x.dtype),
        scratch_shapes=[
            pltpu.VMEM((_NBUF, 2, _G, n_blk * (_KV_ROWS - 2 * _KV_SKEW), dh), _BF16),
            pltpu.VMEM((_NBUF, 2, _G, 2 * n_blk, _KV_SKEW, dh), _BF16),
            pltpu.VMEM((d, hkv * dh), _BF16),
            pltpu.VMEM((hkv * dh, d), _BF16),
            pltpu.VMEM((ff, d), _BF16),
            pltpu.VMEM((ff, d), _BF16),
            pltpu.VMEM((d, 6 * d), _BF16),
            pltpu.VMEM((nb, d), _BF16),
            pltpu.VMEM((nb, d), _BF16),
            pltpu.VMEM((ff,), _BF16),
            pltpu.VMEM((d,), _BF16),
            pltpu.VMEM((1, ff), _F32),
            pltpu.VMEM((hkv, nb, dh), _BF16),
            pltpu.VMEM((hkv, nb, dh), _F32),
            pltpu.SemaphoreType.DMA((_NSEM,)),
        ],
        compiler_params=pltpu.CompilerParams(
            vmem_limit_bytes=48 * 1024 * 1024,
            disable_bounds_checks=True,
            disable_semaphore_checks=True,
        ),
    )(
        A_x.reshape(nb, d),
        A_k_cache.reshape(n_step, _G, sk, dh),
        A_v_cache.reshape(n_step, _G, sk, dh),
        A_k_cache.reshape(n_step, _G, sk // _KV_SKEW, _KV_SKEW, dh),
        A_v_cache.reshape(n_step, _G, sk // _KV_SKEW, _KV_SKEW, dh),
        A_wq, A_wo, B_w1.T, B_b1, B_w2, B_b2, c, w_mod,
    )
    return out.reshape(nb, 1, d)
```

```python
import jax
import jax.numpy as jnp
from jax import lax
import jax.experimental.pallas as pl
import jax.experimental.pallas.tpu as pltpu

_F32 = jnp.float32
_BF16 = jnp.bfloat16
_EPS = 1e-5

_HEADS = 32
_DH = 128
_NSTREAM = 4
_G = _NSTREAM
_NBUF = 3
_AHEAD = 5
_BLOCK = 16
_KV_ROWS = 8 * _BLOCK
_KV_SKEW = 4
_WMOD_SKEW = 8
_FF_ROWS = 16
_FF_CHUNKS = (288, 96, 48)

_S_KV, _S_EDGE = 0, _NBUF
_S_C, _S_X, _S_B1, _S_B2, _S_MOD, _S_Q, _S_O, _S_W1A, _S_W1B, _S_W2 = range(2 * _NBUF, 2 * _NBUF + 10)
_NSEM = _S_W2 + len(_FF_CHUNKS)


def _layernorm(x):
    m = jnp.mean(x, axis=-1, keepdims=True)
    xc = x - m
    v = jnp.mean(xc * xc, axis=-1, keepdims=True)
    return xc * lax.rsqrt(v + _EPS)


def _bursts(t0, t1, width, skew=0, block=_BLOCK):
    out = []
    while t0 < t1:
        end = min(t1, ((t0 + skew) // block + 1) * block - skew)
        rects = []
        while t0 < end:
            r, c = divmod(t0, width)
            nr, nc = ((end - t0) // width, width) if c == 0 and end - t0 >= width else (1, min(width - c, end - t0))
            rects.append((8 * r, 8 * nr, 128 * c, 128 * nc))
            t0 += nr * nc
        out.append(rects)
    return out


def _whole_array(src, dst, sem, skew=0, fine=0):
    width = src.shape[1] // 128
    n_tiles = src.shape[0] // 8 * width
    cuts = [0] + list(range(_BLOCK - skew if skew else _BLOCK, n_tiles, _BLOCK)) + [n_tiles]
    first = [(len(cuts) - 1) * s // (2 * _NSTREAM) for s in range(2 * _NSTREAM + 1)]
    streams = [_bursts(cuts[a], cuts[a + fine], width, skew, _BLOCK // 4) + _bursts(cuts[a + fine], cuts[b], width, skew)
               for a, b in zip(first[:-1], first[1:])]
    queues = [[st[i] for i in range(max(map(len, half))) for st in half if i < len(st)]
              for half in (streams[:_NSTREAM], streams[_NSTREAM:])]
    out = []
    for i in range(max(map(len, queues))):
        for queue in range(2):
            for r, nr, c, nc in queues[queue][i] if i < len(queues[queue]) else ():
                idx = (pl.ds(r, nr), pl.ds(c, nc))
                out.append((src.at[idx], dst.at[idx], sem, queue))
    return out


def _start(copies):
    for src, dst, sem, queue in copies:
        pltpu.make_async_copy(src, dst, sem).start(priority=queue)


def _wait_filled(view, sem):
    pltpu.make_async_copy(view, view, sem).wait()


def _kernel(x_hbm, k_hbm, v_hbm, k4_hbm, v4_hbm, wq_hbm, wo_hbm, w1t_hbm, b1_hbm, w2_hbm, b2_hbm, c_hbm, wmod_hbm,
            o_ref,
            kv_buf, edge_buf, wq_v, wo_v, w1t_v, w2_v, wmod_v, x_v, c_v, b1_v, b2_v, b1_perm, q_scr, o_scr, sem):
    nb, d = x_v.shape
    ff = w2_v.shape[0]
    n_edge = edge_buf.shape[3]
    n_blk = n_edge // 2
    win = n_blk * _KV_ROWS
    row0 = k_hbm.shape[3] - win
    n_c = _HEADS // _G
    n_it = nb * _HEADS
    scale = _DH ** -0.5

    def start_kv(i):
        step = i // _G
        slot = step % _NBUF
        body = _KV_ROWS - 2 * _KV_SKEW
        hint = (lambda v, m: v) if isinstance(i, int) else pl.multiple_of
        for jj in range(n_blk // _G):
            j = (i % _G) * (n_blk // _G) + jj
            for g in range(_G):
                head = (step // n_c, g, step % n_c)
                for which, (src, src4) in enumerate(((k_hbm, k4_hbm), (v_hbm, v4_hbm))):
                    def edge(e):
                        unit = (row0 + (e // 2) * _KV_ROWS + body) // _KV_SKEW + e % 2
                        return (src4.at[head + (pl.ds(unit, 1),)], edge_buf.at[slot, which, g, pl.ds(e, 1)],
                                sem.at[_S_EDGE + slot], 1 - which)
                    _start([edge((2 * j + n_edge - 1) % n_edge),
                            (src.at[head + (pl.ds(hint(row0 + j * _KV_ROWS, _KV_ROWS), body),)],
                             kv_buf.at[slot, which, g, pl.ds(hint(j * body, 8), body)],
                             sem.at[_S_KV + slot], 1 - which),
                            edge(2 * j)])

    ff_stream = ff // _NSTREAM
    assert sum(_FF_CHUNKS) == ff_stream
    ff_pos = [_NSTREAM * sum(_FF_CHUNKS[:k]) for k in range(len(_FF_CHUNKS) + 1)]

    def ff_rows(k, s):
        return s * ff_stream + sum(_FF_CHUNKS[:k]), ff_pos[k] + s * _FF_CHUNKS[k]

    c_cp = pltpu.make_async_copy(c_hbm, c_v, sem.at[_S_C])
    x_cp = pltpu.make_async_copy(x_hbm, x_v, sem.at[_S_X])
    b1_cp = pltpu.make_async_copy(b1_hbm, b1_v, sem.at[_S_B1])
    b2_cp = pltpu.make_async_copy(b2_hbm, b2_v, sem.at[_S_B2])

    _start(_whole_array(wmod_hbm, wmod_v, sem.at[_S_MOD], skew=_WMOD_SKEW, fine=2))
    for cp in (c_cp, x_cp, b1_cp, b2_cp):
        cp.start()
    _start(_whole_array(wq_hbm, wq_v, sem.at[_S_Q]))

    c_cp.wait()
    x_cp.wait()
    b1_cp.wait()
    _wait_filled(wmod_v, sem.at[_S_MOD])
    b1 = b1_v[...].astype(_F32).reshape(1, ff)
    for k, n in enumerate(_FF_CHUNKS):
        for s in range(_NSTREAM):
            r_src, r_dst = ff_rows(k, s)
            b1_perm[:, r_dst:r_dst + n] = b1[:, r_src:r_src + n]
    c = c_v[...].astype(_F32)
    mod = jnp.dot((c * jax.nn.sigmoid(c)).astype(_BF16), wmod_v[...], preferred_element_type=_F32)
    sa, ca, ga, sb, cb, gb = (mod[:, k * d:(k + 1) * d] for k in range(6))
    x = x_v[...].astype(_F32)
    h = (_layernorm(x) * (1.0 + ca) + sa).astype(_BF16)

    for i in range(_AHEAD // 2):
        start_kv(i)
    _wait_filled(wq_v, sem.at[_S_Q])
    q = jnp.dot(h, wq_v[...], preferred_element_type=_F32)
    for hh in range(_HEADS):
        q_scr[hh] = q[:, hh * _DH:(hh + 1) * _DH].astype(_BF16)
    o_scr[...] = jnp.zeros_like(o_scr)
    for i in range(_AHEAD // 2, _AHEAD):
        start_kv(i)

    batch_row = lax.broadcasted_iota(jnp.int32, (nb, _DH), 0)
    wo_copies = _whole_array(wo_hbm, wo_v, sem.at[_S_O])

    def attend(i, carry):
        step = i // _G
        g = i % _G
        slot = step % _NBUF

        @pl.when(i + _AHEAD < n_it)
        def _():
            start_kv(i + _AHEAD)

        for k in range(_AHEAD):
            @pl.when(i + _AHEAD == n_it + k)
            def _():
                _start(wo_copies[len(wo_copies) * k // _AHEAD:len(wo_copies) * (k + 1) // _AHEAD])

        @pl.when(g == 0)
        def _():
            _wait_filled(kv_buf.at[slot], sem.at[_S_KV + slot])
            _wait_filled(edge_buf.at[slot], sem.at[_S_EDGE + slot])

        hh = g * n_c + step % n_c
        k_edge, v_edge = (edge_buf[slot, which, g].reshape(n_edge * _KV_SKEW, _DH) for which in range(2))
        s = jnp.concatenate(
            [lax.dot_general(q_scr[hh], k, (((1,), (1,)), ((), ())), preferred_element_type=_F32)
             for k in (kv_buf[slot, 0, g], k_edge)], axis=-1)
        p = jnp.exp((s - jnp.max(s, axis=-1, keepdims=True)) * scale)
        denom = jnp.sum(p, axis=-1, keepdims=True)
        p = p.astype(_BF16)
        n_body = kv_buf.shape[3]
        o = (jnp.dot(p[:, :n_body], kv_buf[slot, 1, g], preferred_element_type=_F32)
             + jnp.dot(p[:, n_body:], v_edge, preferred_element_type=_F32))
        o_scr[hh] = jnp.where(batch_row == step // n_c, o / denom, o_scr[hh])
        return carry

    lax.fori_loop(0, n_it, attend, 0)

    w1_sems = [sem.at[_S_W1A]] + [sem.at[_S_W1B]] * (len(_FF_CHUNKS) - 1)
    w2_sems = [sem.at[_S_W2 + k] for k in range(len(_FF_CHUNKS))]
    ff_copies = []
    for k, n in enumerate(_FF_CHUNKS):
        for j in range(0, n, _FF_ROWS):
            for s in range(_NSTREAM):
                r_src, r_dst = (pl.ds(r + j, _FF_ROWS) for r in ff_rows(k, s))
                ff_copies.append((w1t_hbm.at[r_src, :], w1t_v.at[r_dst, :], w1_sems[k], 0))
                ff_copies.append((w2_hbm.at[r_src, :], w2_v.at[r_dst, :], w2_sems[k], 1))
    _start(ff_copies[:len(ff_copies) // 2])

    o_all = jnp.concatenate([o_scr[hh] for hh in range(_HEADS)], axis=-1).astype(_BF16)
    _wait_filled(wo_v, sem.at[_S_O])
    x1 = x + ga * jnp.dot(o_all, wo_v[...], preferred_element_type=_F32)
    h2 = (_layernorm(x1) * (1.0 + cb) + sb).astype(_BF16)
    b2_cp.wait()
    _start(ff_copies[len(ff_copies) // 2:])

    def hidden(p0, p1, sm):
        _wait_filled(w1t_v.at[pl.ds(p0, p1 - p0)], sm)
        u = lax.dot_general(h2, w1t_v[p0:p1, :], (((1,), (1,)), ((), ())), preferred_element_type=_F32)
        return jax.nn.gelu(u + b1_perm[:, p0:p1], approximate=True).astype(_BF16)

    def project(act, k):
        p0, p1 = ff_pos[k], ff_pos[k + 1]
        _wait_filled(w2_v.at[pl.ds(p0, p1 - p0)], w2_sems[k])
        return jnp.dot(act, w2_v[p0:p1, :], preferred_element_type=_F32)

    y = b2_v[...].astype(_F32).reshape(1, d) + project(hidden(0, ff_pos[1], w1_sems[0]), 0)
    act = hidden(ff_pos[1], ff, w1_sems[1])
    for k in range(1, len(_FF_CHUNKS)):
        y = y + project(act[:, ff_pos[k] - ff_pos[1]:ff_pos[k + 1] - ff_pos[1]], k)
    o_ref[...] = (x1 + gb * y).astype(o_ref.dtype)


@jax.jit
def pallas_adaLN_cond__sliding_block_cached__dense_activation_gelu__decode_kernel(
    A_x: jax.Array,
    A_k_cache: jax.Array,
    A_v_cache: jax.Array,
    A_wq: jax.Array,
    A_wo: jax.Array,
    B_x: jax.Array,
    B_w1: jax.Array,
    B_b1: jax.Array,
    B_w2: jax.Array,
    B_b2: jax.Array,
    c: jax.Array,
    w_mod: jax.Array,
):
    del B_x
    nb, sq, d = A_x.shape
    _, hkv, sk, dh = A_k_cache.shape
    ff = B_w2.shape[0]
    assert sq == 1 and hkv == _HEADS and dh == _DH
    win = min(4096, max(256, sk // 4))
    assert win % (_G * _KV_ROWS) == 0
    n_blk = win // _KV_ROWS
    heads = (nb, _G, hkv // _G)

    out = pl.pallas_call(
        _kernel,
        in_specs=[pl.BlockSpec(memory_space=pl.ANY)] * 13,
        out_specs=pl.BlockSpec(memory_space=pltpu.VMEM),
        out_shape=jax.ShapeDtypeStruct((nb, d), A_x.dtype),
        scratch_shapes=[
            pltpu.VMEM((_NBUF, 2, _G, n_blk * (_KV_ROWS - 2 * _KV_SKEW), dh), _BF16),
            pltpu.VMEM((_NBUF, 2, _G, 2 * n_blk, _KV_SKEW, dh), _BF16),
            pltpu.VMEM((d, hkv * dh), _BF16),
            pltpu.VMEM((hkv * dh, d), _BF16),
            pltpu.VMEM((ff, d), _BF16),
            pltpu.VMEM((ff, d), _BF16),
            pltpu.VMEM((d, 6 * d), _BF16),
            pltpu.VMEM((nb, d), _BF16),
            pltpu.VMEM((nb, d), _BF16),
            pltpu.VMEM((ff,), _BF16),
            pltpu.VMEM((d,), _BF16),
            pltpu.VMEM((1, ff), _F32),
            pltpu.VMEM((hkv, nb, dh), _BF16),
            pltpu.VMEM((hkv, nb, dh), _F32),
            pltpu.SemaphoreType.DMA((_NSEM,)),
        ],
        compiler_params=pltpu.CompilerParams(
            vmem_limit_bytes=48 * 1024 * 1024,
            disable_bounds_checks=True,
            disable_semaphore_checks=True,
        ),
    )(
        A_x.reshape(nb, d),
        A_k_cache.reshape(heads + (sk, dh)),
        A_v_cache.reshape(heads + (sk, dh)),
        A_k_cache.reshape(heads + (sk // _KV_SKEW, _KV_SKEW, dh)),
        A_v_cache.reshape(heads + (sk // _KV_SKEW, _KV_SKEW, dh)),
        A_wq, A_wo, B_w1.T, B_b1, B_w2, B_b2, c, w_mod,
    )
    return out.reshape(nb, 1, d)
```

```python
import jax
import jax.numpy as jnp
from jax import lax
import jax.experimental.pallas as pl
import jax.experimental.pallas.tpu as pltpu

_F32 = jnp.float32
_BF16 = jnp.bfloat16
_EPS = 1e-5

_HEADS = 32
_DH = 128
_NSTREAM = 4
_G = 8
_STRIDE = 8
_NBUF = 3
_AHEAD = 10
_BLOCK = 16
_KV_ROWS = 8 * _BLOCK
_KV_SKEW = 4
_WMOD_SKEW = 8
_FF_ROWS = 16
_FF_CHUNKS = (288, 96, 48)

_S_KV, _S_EDGE = 0, _NBUF
_S_C, _S_X, _S_B1, _S_B2, _S_MOD, _S_Q, _S_O, _S_W1A, _S_W1B, _S_W2 = range(2 * _NBUF, 2 * _NBUF + 10)
_NSEM = _S_W2 + len(_FF_CHUNKS)


def _layernorm(x):
    m = jnp.mean(x, axis=-1, keepdims=True)
    xc = x - m
    v = jnp.mean(xc * xc, axis=-1, keepdims=True)
    return xc * lax.rsqrt(v + _EPS)


def _bursts(t0, t1, width, skew=0, block=_BLOCK):
    out = []
    while t0 < t1:
        end = min(t1, ((t0 + skew) // block + 1) * block - skew)
        rects = []
        while t0 < end:
            r, c = divmod(t0, width)
            nr, nc = ((end - t0) // width, width) if c == 0 and end - t0 >= width else (1, min(width - c, end - t0))
            rects.append((8 * r, 8 * nr, 128 * c, 128 * nc))
            t0 += nr * nc
        out.append(rects)
    return out


def _whole_array(src, dst, sem, skew=0, fine=0):
    width = src.shape[1] // 128
    n_tiles = src.shape[0] // 8 * width
    cuts = [0] + list(range(_BLOCK - skew if skew else _BLOCK, n_tiles, _BLOCK)) + [n_tiles]
    first = [(len(cuts) - 1) * s // (2 * _NSTREAM) for s in range(2 * _NSTREAM + 1)]
    streams = [_bursts(cuts[a], cuts[a + fine], width, skew, _BLOCK // 4) + _bursts(cuts[a + fine], cuts[b], width, skew)
               for a, b in zip(first[:-1], first[1:])]
    queues = [[st[i] for i in range(max(map(len, half))) for st in half if i < len(st)]
              for half in (streams[:_NSTREAM], streams[_NSTREAM:])]
    out = []
    for i in range(max(map(len, queues))):
        for queue in range(2):
            for r, nr, c, nc in queues[queue][i] if i < len(queues[queue]) else ():
                idx = (pl.ds(r, nr), pl.ds(c, nc))
                out.append((src.at[idx], dst.at[idx], sem, queue))
    return out


def _start(copies):
    for src, dst, sem, queue in copies:
        pltpu.make_async_copy(src, dst, sem).start(priority=queue)


def _wait_filled(view, sem):
    pltpu.make_async_copy(view, view, sem).wait()


def _kernel(x_hbm, k_hbm, v_hbm, k4_hbm, v4_hbm, wq_hbm, wo_hbm, w1t_hbm, b1_hbm, w2_hbm, b2_hbm, c_hbm, wmod_hbm,
            o_ref,
            kv_buf, edge_buf, wq_v, wo_v, w1t_v, w2_v, wmod_v, x_v, c_v, b1_v, b2_v, b1_perm, q_scr, o_scr, sem):
    nb, d = x_v.shape
    ff = w2_v.shape[0]
    n_edge = edge_buf.shape[3]
    n_blk = n_edge // 2
    win = n_blk * _KV_ROWS
    row0 = k_hbm.shape[3] - win
    n_it = nb * _HEADS
    scale = _DH ** -0.5

    def start_kv(i):
        step = i // _G
        slot = step % _NBUF
        body = _KV_ROWS - 2 * _KV_SKEW
        hint = (lambda v, m: v) if isinstance(i, int) else pl.multiple_of
        for jj in range(n_blk // _G):
            j = (i % _G) * (n_blk // _G) + jj
            for g in range(_G):
                pair = (step // _STRIDE, g, step % _STRIDE)
                for which, (src, src4) in enumerate(((k_hbm, k4_hbm), (v_hbm, v4_hbm))):
                    def edge(e):
                        unit = (row0 + (e // 2) * _KV_ROWS + body) // _KV_SKEW + e % 2
                        return (src4.at[pair + (pl.ds(unit, 1),)], edge_buf.at[slot, which, g, pl.ds(e, 1)],
                                sem.at[_S_EDGE + slot], 1 - which)
                    _start([edge((2 * j + n_edge - 1) % n_edge),
                            (src.at[pair + (pl.ds(hint(row0 + j * _KV_ROWS, _KV_ROWS), body),)],
                             kv_buf.at[slot, which, g, pl.ds(hint(j * body, 8), body)],
                             sem.at[_S_KV + slot], 1 - which),
                            edge(2 * j)])

    ff_stream = ff // _NSTREAM
    assert sum(_FF_CHUNKS) == ff_stream
    ff_pos = [_NSTREAM * sum(_FF_CHUNKS[:k]) for k in range(len(_FF_CHUNKS) + 1)]

    def ff_rows(k, s):
        return s * ff_stream + sum(_FF_CHUNKS[:k]), ff_pos[k] + s * _FF_CHUNKS[k]

    w1_sems = [sem.at[_S_W1A]] + [sem.at[_S_W1B]] * (len(_FF_CHUNKS) - 1)
    w2_sems = [sem.at[_S_W2 + k] for k in range(len(_FF_CHUNKS))]
    ff_copies = []
    for k, n in enumerate(_FF_CHUNKS):
        for j in range(0, n, _FF_ROWS):
            for s in range(_NSTREAM):
                r_src, r_dst = (pl.ds(r + j, _FF_ROWS) for r in ff_rows(k, s))
                ff_copies.append((w1t_hbm.at[r_src, :], w1t_v.at[r_dst, :], w1_sems[k], 0))
                ff_copies.append((w2_hbm.at[r_src, :], w2_v.at[r_dst, :], w2_sems[k], 1))

    c_cp = pltpu.make_async_copy(c_hbm, c_v, sem.at[_S_C])
    x_cp = pltpu.make_async_copy(x_hbm, x_v, sem.at[_S_X])
    b1_cp = pltpu.make_async_copy(b1_hbm, b1_v, sem.at[_S_B1])
    b2_cp = pltpu.make_async_copy(b2_hbm, b2_v, sem.at[_S_B2])

    _start(_whole_array(wmod_hbm, wmod_v, sem.at[_S_MOD], skew=_WMOD_SKEW, fine=2))
    for cp in (c_cp, x_cp, b1_cp, b2_cp):
        cp.start()
    _start(_whole_array(wq_hbm, wq_v, sem.at[_S_Q]))

    c_cp.wait()
    x_cp.wait()
    b1_cp.wait()
    _wait_filled(wmod_v, sem.at[_S_MOD])
    b1 = b1_v[...].astype(_F32).reshape(1, ff)
    for k, n in enumerate(_FF_CHUNKS):
        for s in range(_NSTREAM):
            r_src, r_dst = ff_rows(k, s)
            b1_perm[:, r_dst:r_dst + n] = b1[:, r_src:r_src + n]
    c = c_v[...].astype(_F32)
    mod = jnp.dot((c * jax.nn.sigmoid(c)).astype(_BF16), wmod_v[...], preferred_element_type=_F32)
    sa, ca, ga, sb, cb, gb = (mod[:, k * d:(k + 1) * d] for k in range(6))
    x = x_v[...].astype(_F32)
    h = (_layernorm(x) * (1.0 + ca) + sa).astype(_BF16)

    for i in range(_AHEAD // 2):
        start_kv(i)
    _wait_filled(wq_v, sem.at[_S_Q])
    q = jnp.dot(h, wq_v[...], preferred_element_type=_F32)
    for hh in range(_HEADS):
        q_scr[hh] = q[:, hh * _DH:(hh + 1) * _DH].astype(_BF16)
    o_scr[...] = jnp.zeros_like(o_scr)
    for i in range(_AHEAD // 2, _AHEAD):
        start_kv(i)

    batch_row = lax.broadcasted_iota(jnp.int32, (nb, _DH), 0)
    late = _whole_array(wo_hbm, wo_v, sem.at[_S_O]) + ff_copies[:len(ff_copies) // 2]
    sizes = [src.shape[0] * src.shape[1] for src, _, _, _ in late]
    late_part = [sum(sizes[:k]) * _AHEAD // sum(sizes) for k in range(len(late))]

    def attend(i, carry):
        step = i // _G
        g = i % _G
        slot = step % _NBUF

        @pl.when(i + _AHEAD < n_it)
        def _():
            start_kv(i + _AHEAD)

        for k in range(_AHEAD):
            @pl.when(i + _AHEAD == n_it + k)
            def _():
                _start([cp for cp, part in zip(late, late_part) if part == k])

        @pl.when(g == 0)
        def _():
            _wait_filled(kv_buf.at[slot], sem.at[_S_KV + slot])
            _wait_filled(edge_buf.at[slot], sem.at[_S_EDGE + slot])

        pair = ((step // _STRIDE) * _G + g) * _STRIDE + step % _STRIDE
        hh = pair % _HEADS
        k_edge, v_edge = (edge_buf[slot, which, g].reshape(n_edge * _KV_SKEW, _DH) for which in range(2))
        s = jnp.concatenate(
            [lax.dot_general(q_scr[hh], k, (((1,), (1,)), ((), ())), preferred_element_type=_F32)
             for k in (kv_buf[slot, 0, g], k_edge)], axis=-1)
        p = jnp.exp((s - jnp.max(s, axis=-1, keepdims=True)) * scale)
        denom = jnp.sum(p, axis=-1, keepdims=True)
        p = p.astype(_BF16)
        n_body = kv_buf.shape[3]
        o = (jnp.dot(p[:, :n_body], kv_buf[slot, 1, g], preferred_element_type=_F32)
             + jnp.dot(p[:, n_body:], v_edge, preferred_element_type=_F32))
        o_scr[hh] = jnp.where(batch_row == pair // _HEADS, o / denom, o_scr[hh])
        return carry

    lax.fori_loop(0, n_it, attend, 0)

    o_all = jnp.concatenate([o_scr[hh] for hh in range(_HEADS)], axis=-1).astype(_BF16)
    _wait_filled(wo_v, sem.at[_S_O])
    x1 = x + ga * jnp.dot(o_all, wo_v[...], preferred_element_type=_F32)
    h2 = (_layernorm(x1) * (1.0 + cb) + sb).astype(_BF16)
    b2_cp.wait()
    _start(ff_copies[len(ff_copies) // 2:])

    def hidden(p0, p1, sm):
        _wait_filled(w1t_v.at[pl.ds(p0, p1 - p0)], sm)
        u = lax.dot_general(h2, w1t_v[p0:p1, :], (((1,), (1,)), ((), ())), preferred_element_type=_F32)
        return jax.nn.gelu(u + b1_perm[:, p0:p1], approximate=True).astype(_BF16)

    def project(act, k):
        p0, p1 = ff_pos[k], ff_pos[k + 1]
        _wait_filled(w2_v.at[pl.ds(p0, p1 - p0)], w2_sems[k])
        return jnp.dot(act, w2_v[p0:p1, :], preferred_element_type=_F32)

    y = b2_v[...].astype(_F32).reshape(1, d) + project(hidden(0, ff_pos[1], w1_sems[0]), 0)
    act = hidden(ff_pos[1], ff, w1_sems[1])
    for k in range(1, len(_FF_CHUNKS)):
        y = y + project(act[:, ff_pos[k] - ff_pos[1]:ff_pos[k + 1] - ff_pos[1]], k)
    o_ref[...] = (x1 + gb * y).astype(o_ref.dtype)


@jax.jit
def pallas_adaLN_cond__sliding_block_cached__dense_activation_gelu__decode_kernel(
    A_x: jax.Array,
    A_k_cache: jax.Array,
    A_v_cache: jax.Array,
    A_wq: jax.Array,
    A_wo: jax.Array,
    B_x: jax.Array,
    B_w1: jax.Array,
    B_b1: jax.Array,
    B_w2: jax.Array,
    B_b2: jax.Array,
    c: jax.Array,
    w_mod: jax.Array,
):
    del B_x
    nb, sq, d = A_x.shape
    _, hkv, sk, dh = A_k_cache.shape
    ff = B_w2.shape[0]
    assert sq == 1 and hkv == _HEADS and dh == _DH
    win = min(4096, max(256, sk // 4))
    assert win % (_G * _KV_ROWS) == 0
    n_blk = win // _KV_ROWS
    pairs = (nb * hkv // (_G * _STRIDE), _G, _STRIDE)

    out = pl.pallas_call(
        _kernel,
        in_specs=[pl.BlockSpec(memory_space=pl.ANY)] * 13,
        out_specs=pl.BlockSpec(memory_space=pltpu.VMEM),
        out_shape=jax.ShapeDtypeStruct((nb, d), A_x.dtype),
        scratch_shapes=[
            pltpu.VMEM((_NBUF, 2, _G, n_blk * (_KV_ROWS - 2 * _KV_SKEW), dh), _BF16),
            pltpu.VMEM((_NBUF, 2, _G, 2 * n_blk, _KV_SKEW, dh), _BF16),
            pltpu.VMEM((d, hkv * dh), _BF16),
            pltpu.VMEM((hkv * dh, d), _BF16),
            pltpu.VMEM((ff, d), _BF16),
            pltpu.VMEM((ff, d), _BF16),
            pltpu.VMEM((d, 6 * d), _BF16),
            pltpu.VMEM((nb, d), _BF16),
            pltpu.VMEM((nb, d), _BF16),
            pltpu.VMEM((ff,), _BF16),
            pltpu.VMEM((d,), _BF16),
            pltpu.VMEM((1, ff), _F32),
            pltpu.VMEM((hkv, nb, dh), _BF16),
            pltpu.VMEM((hkv, nb, dh), _F32),
            pltpu.SemaphoreType.DMA((_NSEM,)),
        ],
        compiler_params=pltpu.CompilerParams(
            vmem_limit_bytes=64 * 1024 * 1024,
            disable_bounds_checks=True,
            disable_semaphore_checks=True,
        ),
    )(
        A_x.reshape(nb, d),
        A_k_cache.reshape(pairs + (sk, dh)),
        A_v_cache.reshape(pairs + (sk, dh)),
        A_k_cache.reshape(pairs + (sk // _KV_SKEW, _KV_SKEW, dh)),
        A_v_cache.reshape(pairs + (sk // _KV_SKEW, _KV_SKEW, dh)),
        A_wq, A_wo, B_w1.T, B_b1, B_w2, B_b2, c, w_mod,
    )
    return out.reshape(nb, 1, d)
```

```python
import jax
import jax.numpy as jnp
from jax import lax
import jax.experimental.pallas as pl
import jax.experimental.pallas.tpu as pltpu

_F32 = jnp.float32
_BF16 = jnp.bfloat16
_EPS = 1e-5

_HEADS = 32
_DH = 128
_NSTREAM = 4
_G = 8
_STRIDE = 8
_NBUF = 3
_AHEAD = 10
_BLOCK = 16
_KV_ROWS = 8 * _BLOCK
_KV_SKEW = 4
_WMOD_SKEW = 8
_FF_ROWS = 16
_FF_CHUNKS = (288, 96, 48)

_S_KV, _S_EDGE = 0, _NBUF
_S_C, _S_X, _S_B1, _S_B2, _S_MOD, _S_Q, _S_O, _S_W1A, _S_W1B, _S_W2 = range(2 * _NBUF, 2 * _NBUF + 10)
_NSEM = _S_W2 + len(_FF_CHUNKS)


def _layernorm(x):
    m = jnp.mean(x, axis=-1, keepdims=True)
    xc = x - m
    v = jnp.mean(xc * xc, axis=-1, keepdims=True)
    return xc * lax.rsqrt(v + _EPS)


def _whole_array(src, dst, sem, skew=0):
    width = src.shape[1] // 128
    n_tiles = src.shape[0] // 8 * width
    blocks, t = [], 0
    while t < n_tiles:
        end = min(n_tiles, ((t + skew) // _BLOCK + 1) * _BLOCK - skew)
        blocks.append([])
        while t < end:
            r, c = divmod(t, width)
            nr, nc = ((end - t) // width, width) if c == 0 and end - t >= width else (1, min(width - c, end - t))
            blocks[-1].append((8 * r, 8 * nr, 128 * c, 128 * nc))
            t += nr * nc
    n = 2 * _NSTREAM
    streams = [blocks[len(blocks) * s // n:len(blocks) * (s + 1) // n] for s in range(n)]
    queues = [[st[i] for i in range(max(map(len, half))) for st in half if i < len(st)]
              for half in (streams[:_NSTREAM], streams[_NSTREAM:])]
    out = []
    for i in range(max(map(len, queues))):
        for queue in range(2):
            for r, nr, c, nc in queues[queue][i] if i < len(queues[queue]) else ():
                idx = (pl.ds(r, nr), pl.ds(c, nc))
                out.append((src.at[idx], dst.at[idx], sem, queue))
    return out


def _start(copies):
    for src, dst, sem, queue in copies:
        pltpu.make_async_copy(src, dst, sem).start(priority=queue)


def _wait_filled(view, sem):
    pltpu.make_async_copy(view, view, sem).wait()


def _kernel(x_hbm, k_hbm, v_hbm, k4_hbm, v4_hbm, wq_hbm, wo_hbm, w1t_hbm, b1_hbm, w2_hbm, b2_hbm, c_hbm, wmod_hbm,
            o_ref,
            kv_buf, edge_buf, wq_v, wo_v, w1t_v, w2_v, wmod_v, x_v, c_v, b1_v, b2_v, b1_perm, q_scr, o_scr, sem):
    nb, d = x_v.shape
    ff = w2_v.shape[0]
    n_edge = edge_buf.shape[3]
    n_blk = n_edge // 2
    win = n_blk * _KV_ROWS
    row0 = k_hbm.shape[3] - win
    n_it = nb * _HEADS
    scale = _DH ** -0.5

    def start_kv(i):
        step = i // _G
        slot = step % _NBUF
        body = _KV_ROWS - 2 * _KV_SKEW
        hint = (lambda v, m: v) if isinstance(i, int) else pl.multiple_of
        for jj in range(n_blk // _G):
            j = (i % _G) * (n_blk // _G) + jj
            for g in range(_G):
                pair = (step // _STRIDE, g, step % _STRIDE)
                for which, (src, src4) in enumerate(((k_hbm, k4_hbm), (v_hbm, v4_hbm))):
                    def edge(e):
                        unit = (row0 + (e // 2) * _KV_ROWS + body) // _KV_SKEW + e % 2
                        return (src4.at[pair + (pl.ds(unit, 1),)], edge_buf.at[slot, which, g, pl.ds(e, 1)],
                                sem.at[_S_EDGE + slot], 1 - which)
                    _start([edge((2 * j + n_edge - 1) % n_edge),
                            (src.at[pair + (pl.ds(hint(row0 + j * _KV_ROWS, _KV_ROWS), body),)],
                             kv_buf.at[slot, which, g, pl.ds(hint(j * body, 8), body)],
                             sem.at[_S_KV + slot], 1 - which),
                            edge(2 * j)])

    ff_stream = ff // _NSTREAM
    assert sum(_FF_CHUNKS) == ff_stream
    ff_pos = [_NSTREAM * sum(_FF_CHUNKS[:k]) for k in range(len(_FF_CHUNKS) + 1)]

    def ff_rows(k, s):
        return s * ff_stream + sum(_FF_CHUNKS[:k]), ff_pos[k] + s * _FF_CHUNKS[k]

    w1_sems = [sem.at[_S_W1A]] + [sem.at[_S_W1B]] * (len(_FF_CHUNKS) - 1)
    w2_sems = [sem.at[_S_W2 + k] for k in range(len(_FF_CHUNKS))]
    ff_copies = []
    for k, n in enumerate(_FF_CHUNKS):
        for j in range(0, n, _FF_ROWS):
            for s in range(_NSTREAM):
                r_src, r_dst = (pl.ds(r + j, _FF_ROWS) for r in ff_rows(k, s))
                ff_copies.append((w1t_hbm.at[r_src, :], w1t_v.at[r_dst, :], w1_sems[k], 0))
                ff_copies.append((w2_hbm.at[r_src, :], w2_v.at[r_dst, :], w2_sems[k], 1))

    c_cp = pltpu.make_async_copy(c_hbm, c_v, sem.at[_S_C])
    x_cp = pltpu.make_async_copy(x_hbm, x_v, sem.at[_S_X])
    b1_cp = pltpu.make_async_copy(b1_hbm, b1_v, sem.at[_S_B1])
    b2_cp = pltpu.make_async_copy(b2_hbm, b2_v, sem.at[_S_B2])

    for i in range(2):
        start_kv(i)
    _start(_whole_array(wmod_hbm, wmod_v, sem.at[_S_MOD], skew=_WMOD_SKEW))
    for cp in (c_cp, x_cp, b1_cp, b2_cp):
        cp.start()
    _start(_whole_array(wq_hbm, wq_v, sem.at[_S_Q]))

    c_cp.wait()
    x_cp.wait()
    b1_cp.wait()
    _wait_filled(wmod_v, sem.at[_S_MOD])
    b1 = b1_v[...].astype(_F32).reshape(1, ff)
    for k, n in enumerate(_FF_CHUNKS):
        for s in range(_NSTREAM):
            r_src, r_dst = ff_rows(k, s)
            b1_perm[:, r_dst:r_dst + n] = b1[:, r_src:r_src + n]
    c = c_v[...].astype(_F32)
    mod = jnp.dot((c * jax.nn.sigmoid(c)).astype(_BF16), wmod_v[...], preferred_element_type=_F32)
    sa, ca, ga, sb, cb, gb = (mod[:, k * d:(k + 1) * d] for k in range(6))
    x = x_v[...].astype(_F32)
    h = (_layernorm(x) * (1.0 + ca) + sa).astype(_BF16)

    for i in range(2, _AHEAD // 2):
        start_kv(i)
    _wait_filled(wq_v, sem.at[_S_Q])
    q = jnp.dot(h, wq_v[...], preferred_element_type=_F32)
    for hh in range(_HEADS):
        q_scr[hh] = q[:, hh * _DH:(hh + 1) * _DH].astype(_BF16)
    o_scr[...] = jnp.zeros_like(o_scr)
    for i in range(_AHEAD // 2, _AHEAD):
        start_kv(i)

    batch_row = lax.broadcasted_iota(jnp.int32, (nb, _DH), 0)
    late = _whole_array(wo_hbm, wo_v, sem.at[_S_O]) + ff_copies[:len(ff_copies) // 2]
    sizes = [src.shape[0] * src.shape[1] for src, _, _, _ in late]
    late_part = [sum(sizes[:k]) * _AHEAD // sum(sizes) for k in range(len(late))]

    def attend(i, carry):
        step = i // _G
        g = i % _G
        slot = step % _NBUF

        @pl.when(i + _AHEAD < n_it)
        def _():
            start_kv(i + _AHEAD)

        for k in range(_AHEAD):
            @pl.when(i + _AHEAD == n_it + k)
            def _():
                _start([cp for cp, part in zip(late, late_part) if part == k])

        @pl.when(g == 0)
        def _():
            _wait_filled(kv_buf.at[slot], sem.at[_S_KV + slot])
            _wait_filled(edge_buf.at[slot], sem.at[_S_EDGE + slot])

        pair = ((step // _STRIDE) * _G + g) * _STRIDE + step % _STRIDE
        hh = pair % _HEADS
        k_edge, v_edge = (edge_buf[slot, which, g].reshape(n_edge * _KV_SKEW, _DH) for which in range(2))
        s = jnp.concatenate(
            [lax.dot_general(q_scr[hh], k, (((1,), (1,)), ((), ())), preferred_element_type=_F32)
             for k in (kv_buf[slot, 0, g], k_edge)], axis=-1)
        p = jnp.exp((s - jnp.max(s, axis=-1, keepdims=True)) * scale)
        denom = jnp.sum(p, axis=-1, keepdims=True)
        p = p.astype(_BF16)
        n_body = kv_buf.shape[3]
        o = (jnp.dot(p[:, :n_body], kv_buf[slot, 1, g], preferred_element_type=_F32)
             + jnp.dot(p[:, n_body:], v_edge, preferred_element_type=_F32))
        o_scr[hh] = jnp.where(batch_row == pair // _HEADS, o / denom, o_scr[hh])
        return carry

    lax.fori_loop(0, n_it, attend, 0)

    o_all = jnp.concatenate([o_scr[hh] for hh in range(_HEADS)], axis=-1).astype(_BF16)
    _wait_filled(wo_v, sem.at[_S_O])
    x1 = x + ga * jnp.dot(o_all, wo_v[...], preferred_element_type=_F32)
    h2 = (_layernorm(x1) * (1.0 + cb) + sb).astype(_BF16)
    b2_cp.wait()
    _start(ff_copies[len(ff_copies) // 2:])

    def hidden(p0, p1, sm):
        _wait_filled(w1t_v.at[pl.ds(p0, p1 - p0)], sm)
        u = lax.dot_general(h2, w1t_v[p0:p1, :], (((1,), (1,)), ((), ())), preferred_element_type=_F32)
        return jax.nn.gelu(u + b1_perm[:, p0:p1], approximate=True).astype(_BF16)

    def project(act, k):
        p0, p1 = ff_pos[k], ff_pos[k + 1]
        _wait_filled(w2_v.at[pl.ds(p0, p1 - p0)], w2_sems[k])
        return jnp.dot(act, w2_v[p0:p1, :], preferred_element_type=_F32)

    y = b2_v[...].astype(_F32).reshape(1, d) + project(hidden(0, ff_pos[1], w1_sems[0]), 0)
    act = hidden(ff_pos[1], ff, w1_sems[1])
    for k in range(1, len(_FF_CHUNKS)):
        y = y + project(act[:, ff_pos[k] - ff_pos[1]:ff_pos[k + 1] - ff_pos[1]], k)
    o_ref[...] = (x1 + gb * y).astype(o_ref.dtype)


@jax.jit
def pallas_adaLN_cond__sliding_block_cached__dense_activation_gelu__decode_kernel(
    A_x: jax.Array,
    A_k_cache: jax.Array,
    A_v_cache: jax.Array,
    A_wq: jax.Array,
    A_wo: jax.Array,
    B_x: jax.Array,
    B_w1: jax.Array,
    B_b1: jax.Array,
    B_w2: jax.Array,
    B_b2: jax.Array,
    c: jax.Array,
    w_mod: jax.Array,
):
    del B_x
    nb, sq, d = A_x.shape
    _, hkv, sk, dh = A_k_cache.shape
    ff = B_w2.shape[0]
    assert sq == 1 and hkv == _HEADS and dh == _DH
    win = min(4096, max(256, sk // 4))
    assert win % (_G * _KV_ROWS) == 0
    n_blk = win // _KV_ROWS
    pairs = (nb * hkv // (_G * _STRIDE), _G, _STRIDE)

    out = pl.pallas_call(
        _kernel,
        in_specs=[pl.BlockSpec(memory_space=pl.ANY)] * 13,
        out_specs=pl.BlockSpec(memory_space=pltpu.VMEM),
        out_shape=jax.ShapeDtypeStruct((nb, d), A_x.dtype),
        scratch_shapes=[
            pltpu.VMEM((_NBUF, 2, _G, n_blk * (_KV_ROWS - 2 * _KV_SKEW), dh), _BF16),
            pltpu.VMEM((_NBUF, 2, _G, 2 * n_blk, _KV_SKEW, dh), _BF16),
            pltpu.VMEM((d, hkv * dh), _BF16),
            pltpu.VMEM((hkv * dh, d), _BF16),
            pltpu.VMEM((ff, d), _BF16),
            pltpu.VMEM((ff, d), _BF16),
            pltpu.VMEM((d, 6 * d), _BF16),
            pltpu.VMEM((nb, d), _BF16),
            pltpu.VMEM((nb, d), _BF16),
            pltpu.VMEM((ff,), _BF16),
            pltpu.VMEM((d,), _BF16),
            pltpu.VMEM((1, ff), _F32),
            pltpu.VMEM((hkv, nb, dh), _BF16),
            pltpu.VMEM((hkv, nb, dh), _F32),
            pltpu.SemaphoreType.DMA((_NSEM,)),
        ],
        compiler_params=pltpu.CompilerParams(
            vmem_limit_bytes=64 * 1024 * 1024,
            disable_bounds_checks=True,
            disable_semaphore_checks=True,
        ),
    )(
        A_x.reshape(nb, d),
        A_k_cache.reshape(pairs + (sk, dh)),
        A_v_cache.reshape(pairs + (sk, dh)),
        A_k_cache.reshape(pairs + (sk // _KV_SKEW, _KV_SKEW, dh)),
        A_v_cache.reshape(pairs + (sk // _KV_SKEW, _KV_SKEW, dh)),
        A_wq, A_wo, B_w1.T, B_b1, B_w2, B_b2, c, w_mod,
    )
    return out.reshape(nb, 1, d)
```

```python
import jax
import jax.numpy as jnp
from jax import lax
import jax.experimental.pallas as pl
import jax.experimental.pallas.tpu as pltpu

_F32 = jnp.float32
_BF16 = jnp.bfloat16
_EPS = 1e-5

_HEADS = 32
_DH = 128
_NSTREAM = 4
_G = 8
_STRIDE = 8
_NBUF = 3
_AHEAD = 11
_BLOCK = 16
_KV_ROWS = 8 * _BLOCK
_WMOD_SKEW = 8
_FF_ROWS = 16
_FF_CHUNKS = (288, 96, 48)

_S_KV = 0
_S_C, _S_X, _S_B1, _S_B2, _S_MOD, _S_Q, _S_O, _S_W1A, _S_W1B, _S_W2 = range(_NBUF, _NBUF + 10)
_NSEM = _S_W2 + len(_FF_CHUNKS)


def _layernorm(x):
    m = jnp.mean(x, axis=-1, keepdims=True)
    xc = x - m
    v = jnp.mean(xc * xc, axis=-1, keepdims=True)
    return xc * lax.rsqrt(v + _EPS)


def _whole_array(src, dst, sem, skew=0):
    width = src.shape[1] // 128
    n_tiles = src.shape[0] // 8 * width
    blocks, t = [], 0
    while t < n_tiles:
        end = min(n_tiles, ((t + skew) // _BLOCK + 1) * _BLOCK - skew)
        blocks.append([])
        while t < end:
            r, c = divmod(t, width)
            nr, nc = ((end - t) // width, width) if c == 0 and end - t >= width else (1, min(width - c, end - t))
            blocks[-1].append((8 * r, 8 * nr, 128 * c, 128 * nc))
            t += nr * nc
    n = 2 * _NSTREAM
    streams = [blocks[len(blocks) * s // n:len(blocks) * (s + 1) // n] for s in range(n)]
    queues = [[st[i] for i in range(max(map(len, half))) for st in half if i < len(st)]
              for half in (streams[:_NSTREAM], streams[_NSTREAM:])]
    out = []
    for i in range(max(map(len, queues))):
        for queue in range(2):
            for r, nr, c, nc in queues[queue][i] if i < len(queues[queue]) else ():
                idx = (pl.ds(r, nr), pl.ds(c, nc))
                out.append((src.at[idx], dst.at[idx], sem, queue))
    return out


def _start(copies):
    for src, dst, sem, queue in copies:
        pltpu.make_async_copy(src, dst, sem).start(priority=queue)


def _wait_filled(view, sem):
    pltpu.make_async_copy(view, view, sem).wait()


def _kernel(x_hbm, k_hbm, v_hbm, wq_hbm, wo_hbm, w1t_hbm, b1_hbm, w2_hbm, b2_hbm, c_hbm, wmod_hbm,
            o_ref,
            kv_buf, wq_v, wo_v, w1t_v, w2_v, wmod_v, x_v, c_v, b1_v, b2_v, b1_perm, q_scr, o_scr, sem):
    nb, d = x_v.shape
    ff = w2_v.shape[0]
    win = kv_buf.shape[3]
    row0 = k_hbm.shape[3] - win
    n_it = nb * _HEADS
    scale = _DH ** -0.5

    def start_kv(i, n_rows=_KV_ROWS):
        step = i // _G
        slot = step % _NBUF
        outer, inner = step // _STRIDE, step % _STRIDE
        kv_sem = sem.at[_S_KV + slot]
        for j in range(0, win // _G, n_rows):
            r = (i % _G) * (win // _G) + j
            if not isinstance(r, int):
                r = pl.multiple_of(r, n_rows)
            src_rows, dst_rows = pl.ds(row0 + r, n_rows), pl.ds(r, n_rows)
            for g in range(_G):
                for which, src in enumerate((k_hbm, v_hbm)):
                    pltpu.make_async_copy(src.at[outer, g, inner, src_rows], kv_buf.at[slot, which, g, dst_rows],
                                          kv_sem).start(priority=1 - which)

    ff_stream = ff // _NSTREAM
    assert sum(_FF_CHUNKS) == ff_stream
    ff_pos = [_NSTREAM * sum(_FF_CHUNKS[:k]) for k in range(len(_FF_CHUNKS) + 1)]

    def ff_rows(k, s):
        return s * ff_stream + sum(_FF_CHUNKS[:k]), ff_pos[k] + s * _FF_CHUNKS[k]

    w1_sems = [sem.at[_S_W1A]] + [sem.at[_S_W1B]] * (len(_FF_CHUNKS) - 1)
    w2_sems = [sem.at[_S_W2 + k] for k in range(len(_FF_CHUNKS))]
    ff_copies = []
    for k, n in enumerate(_FF_CHUNKS):
        for j in range(0, n, _FF_ROWS):
            for s in range(_NSTREAM):
                r_src, r_dst = (pl.ds(r + j, _FF_ROWS) for r in ff_rows(k, s))
                ff_copies.append((w1t_hbm.at[r_src, :], w1t_v.at[r_dst, :], w1_sems[k], 0))
                ff_copies.append((w2_hbm.at[r_src, :], w2_v.at[r_dst, :], w2_sems[k], 1))

    c_cp = pltpu.make_async_copy(c_hbm, c_v, sem.at[_S_C])
    x_cp = pltpu.make_async_copy(x_hbm, x_v, sem.at[_S_X])
    b1_cp = pltpu.make_async_copy(b1_hbm, b1_v, sem.at[_S_B1])
    b2_cp = pltpu.make_async_copy(b2_hbm, b2_v, sem.at[_S_B2])

    start_kv(0, _KV_ROWS // 4)
    _start(_whole_array(wmod_hbm, wmod_v, sem.at[_S_MOD], skew=_WMOD_SKEW))
    for cp in (c_cp, x_cp, b1_cp, b2_cp):
        cp.start()
    _start(_whole_array(wq_hbm, wq_v, sem.at[_S_Q]))

    c_cp.wait()
    x_cp.wait()
    b1_cp.wait()
    _wait_filled(wmod_v, sem.at[_S_MOD])
    b1 = b1_v[...].astype(_F32).reshape(1, ff)
    for k, n in enumerate(_FF_CHUNKS):
        for s in range(_NSTREAM):
            r_src, r_dst = ff_rows(k, s)
            b1_perm[:, r_dst:r_dst + n] = b1[:, r_src:r_src + n]
    c = c_v[...].astype(_F32)
    mod = jnp.dot((c * jax.nn.sigmoid(c)).astype(_BF16), wmod_v[...], preferred_element_type=_F32)
    sa, ca, ga, sb, cb, gb = (mod[:, k * d:(k + 1) * d] for k in range(6))
    x = x_v[...].astype(_F32)
    h = (_layernorm(x) * (1.0 + ca) + sa).astype(_BF16)

    for i in range(1, _AHEAD // 2):
        start_kv(i)
    _wait_filled(wq_v, sem.at[_S_Q])
    q = jnp.dot(h, wq_v[...], preferred_element_type=_F32)
    for hh in range(_HEADS):
        q_scr[hh] = q[:, hh * _DH:(hh + 1) * _DH].astype(_BF16)
    o_scr[...] = jnp.zeros_like(o_scr)
    for i in range(_AHEAD // 2, _AHEAD):
        start_kv(i)

    batch_row = lax.broadcasted_iota(jnp.int32, (nb, _DH), 0)
    late = _whole_array(wo_hbm, wo_v, sem.at[_S_O]) + ff_copies[:len(ff_copies) // 2]
    sizes = [src.shape[0] * src.shape[1] for src, _, _, _ in late]
    late_part = [sum(sizes[:k]) * _AHEAD // sum(sizes) for k in range(len(late))]

    def attend(i, carry):
        step = i // _G
        g = i % _G
        slot = step % _NBUF

        @pl.when(i + _AHEAD < n_it)
        def _():
            start_kv(i + _AHEAD)

        for k in range(_AHEAD):
            @pl.when(i + _AHEAD == n_it + k)
            def _():
                _start([cp for cp, part in zip(late, late_part) if part == k])

        @pl.when(g == 0)
        def _():
            _wait_filled(kv_buf.at[slot], sem.at[_S_KV + slot])

        pair = ((step // _STRIDE) * _G + g) * _STRIDE + step % _STRIDE
        hh = pair % _HEADS
        s = lax.dot_general(q_scr[hh], kv_buf[slot, 0, g], (((1,), (1,)), ((), ())),
                            preferred_element_type=_F32)
        p = jnp.exp((s - jnp.max(s, axis=-1, keepdims=True)) * scale)
        denom = jnp.sum(p, axis=-1, keepdims=True)
        o = jnp.dot(p.astype(_BF16), kv_buf[slot, 1, g], preferred_element_type=_F32)
        o_scr[hh] = jnp.where(batch_row == pair // _HEADS, o / denom, o_scr[hh])
        return carry

    lax.fori_loop(0, n_it, attend, 0)

    o_all = jnp.concatenate([o_scr[hh] for hh in range(_HEADS)], axis=-1).astype(_BF16)
    _wait_filled(wo_v, sem.at[_S_O])
    x1 = x + ga * jnp.dot(o_all, wo_v[...], preferred_element_type=_F32)
    h2 = (_layernorm(x1) * (1.0 + cb) + sb).astype(_BF16)
    b2_cp.wait()
    _start(ff_copies[len(ff_copies) // 2:])

    def hidden(p0, p1, sm):
        _wait_filled(w1t_v.at[pl.ds(p0, p1 - p0)], sm)
        u = lax.dot_general(h2, w1t_v[p0:p1, :], (((1,), (1,)), ((), ())), preferred_element_type=_F32)
        return jax.nn.gelu(u + b1_perm[:, p0:p1], approximate=True).astype(_BF16)

    def project(act, k):
        p0, p1 = ff_pos[k], ff_pos[k + 1]
        _wait_filled(w2_v.at[pl.ds(p0, p1 - p0)], w2_sems[k])
        return jnp.dot(act, w2_v[p0:p1, :], preferred_element_type=_F32)

    y = b2_v[...].astype(_F32).reshape(1, d) + project(hidden(0, ff_pos[1], w1_sems[0]), 0)
    act = hidden(ff_pos[1], ff, w1_sems[1])
    for k in range(1, len(_FF_CHUNKS)):
        y = y + project(act[:, ff_pos[k] - ff_pos[1]:ff_pos[k + 1] - ff_pos[1]], k)
    o_ref[...] = (x1 + gb * y).astype(o_ref.dtype)


@jax.jit
def pallas_adaLN_cond__sliding_block_cached__dense_activation_gelu__decode_kernel(
    A_x: jax.Array,
    A_k_cache: jax.Array,
    A_v_cache: jax.Array,
    A_wq: jax.Array,
    A_wo: jax.Array,
    B_x: jax.Array,
    B_w1: jax.Array,
    B_b1: jax.Array,
    B_w2: jax.Array,
    B_b2: jax.Array,
    c: jax.Array,
    w_mod: jax.Array,
):
    del B_x
    nb, sq, d = A_x.shape
    _, hkv, sk, dh = A_k_cache.shape
    ff = B_w2.shape[0]
    assert sq == 1 and hkv == _HEADS and dh == _DH
    win = min(4096, max(256, sk // 4))
    assert win % (_G * _KV_ROWS) == 0
    pairs = (nb * hkv // (_G * _STRIDE), _G, _STRIDE)

    out = pl.pallas_call(
        _kernel,
        in_specs=[pl.BlockSpec(memory_space=pl.ANY)] * 11,
        out_specs=pl.BlockSpec(memory_space=pltpu.VMEM),
        out_shape=jax.ShapeDtypeStruct((nb, d), A_x.dtype),
        scratch_shapes=[
            pltpu.VMEM((_NBUF, 2, _G, win, dh), _BF16),
            pltpu.VMEM((d, hkv * dh), _BF16),
            pltpu.VMEM((hkv * dh, d), _BF16),
            pltpu.VMEM((ff, d), _BF16),
            pltpu.VMEM((ff, d), _BF16),
            pltpu.VMEM((d, 6 * d), _BF16),
            pltpu.VMEM((nb, d), _BF16),
            pltpu.VMEM((nb, d), _BF16),
            pltpu.VMEM((ff,), _BF16),
            pltpu.VMEM((d,), _BF16),
            pltpu.VMEM((1, ff), _F32),
            pltpu.VMEM((hkv, nb, dh), _BF16),
            pltpu.VMEM((hkv, nb, dh), _F32),
            pltpu.SemaphoreType.DMA((_NSEM,)),
        ],
        compiler_params=pltpu.CompilerParams(
            vmem_limit_bytes=64 * 1024 * 1024,
            disable_bounds_checks=True,
            disable_semaphore_checks=True,
        ),
    )(
        A_x.reshape(nb, d),
        A_k_cache.reshape(pairs + (sk, dh)),
        A_v_cache.reshape(pairs + (sk, dh)),
        A_wq, A_wo, B_w1.T, B_b1, B_w2, B_b2, c, w_mod,
    )
    return out.reshape(nb, 1, d)
```
